```python
import os as _os
_os.environ.setdefault("JAX_PLATFORMS", "cpu")
import jax
import jax.numpy as jnp

def _softmax(x, axis=-1):
    return jax.nn.softmax(x, axis=axis)
def _gelu(x):
    return jax.nn.gelu(x, approximate=True)
def _silu(x):
    return jax.nn.silu(x)
def _sigmoid(x):
    return jax.nn.sigmoid(x)
def _layernorm(x, axis=-1, eps=1e-5):
    m = jnp.mean(x, axis=axis, keepdims=True)
    v = jnp.var(x, axis=axis, keepdims=True)
    return (x - m) / jnp.sqrt(v + eps)
def _scatter_add(tgt, idx, src, axis=0):
    return tgt.at[idx].add(src)
def _segment_sum(src, seg, n):
    return jax.ops.segment_sum(src, seg, n)
class _Rng:
    def __init__(self, key):
        self._k = key
    def _next(self):
        self._k, sub = jax.random.split(self._k)
        return sub
    def normal(self, shape):
        return jax.random.normal(self._next(), shape, dtype=jnp.bfloat16)
    def randint(self, lo, hi, shape):
        return jax.random.randint(self._next(), shape, lo, hi, dtype=jnp.int32)
    def uniform(self, shape, lo=0.0, hi=1.0):
        return jax.random.uniform(self._next(), shape, jnp.bfloat16, lo, hi)
    def permutation(self, n):
        return jax.random.permutation(self._next(), n)


kernel_name = 'interleave_layers__linear_attn_block__mha_block__prompt'

def setup_inputs():
    _rng = _Rng(jax.random.key(int.from_bytes(__import__("os").urandom(4), "little")))
    _w = (lambda a: (lambda t: t.astype(jnp.bfloat16) if jnp.issubdtype(t.dtype, jnp.floating) else t)(jnp.asarray(a)))
    def _A_setup():
        B, S, D = 1, 2048, 1024
        return {
            "x": _w((lambda *s: _rng.normal(s) * 0.05)(B, S, D)),
            "wqkv": _w((lambda *s: _rng.normal(s) * 0.1)(D, 3 * D)),
            "wo": _w((lambda *s: _rng.normal(s) * 0.1)(D, D)),
        }
    _A_in = _A_setup()

    def _B_setup():
        B, S, D, H = 1, 2048, 1024, 32
        return {
            "x": _w((lambda *s: _rng.normal(s) * 0.05)(B, S, D)),
            "wqkv": _w((lambda *s: _rng.normal(s) * 0.1)(D, 3 * D)),
            "wo": _w((lambda *s: _rng.normal(s) * 0.05)(D, D)),
        }
    _B_in = _B_setup()

    return {
        "A_x": _A_in["x"],
        "A_wqkv": _A_in["wqkv"],
        "A_wo": _A_in["wo"],
        "B_x": _B_in["x"],
        "B_wqkv": _B_in["wqkv"],
        "B_wo": _B_in["wo"],
    }

def reference(A_x, A_wqkv, A_wo, B_x, B_wqkv, B_wo):
    def _A_ref(x, wqkv, wo):
        B, S, D = x.shape
        H = 32; Dh = D // H
        qkv = (lambda x, *d: x.transpose(*d))((x @ wqkv).reshape(B, S, 3, H, Dh), 2, 0, 3, 1, 4)
        q, k, v = qkv[0], qkv[1], qkv[2]
        phi = lambda t: jnp.where(t > 0, t + 1, jnp.exp(t)) + 1e-6
        pq, pk = phi(q), phi(k)
        kv = jnp.einsum("bhsd,bhse->bhde", pk, v)
        z = jnp.einsum("bhsd->bhd", pk)
        num = jnp.einsum("bhqd,bhde->bhqe", pq, kv)
        den = jnp.einsum("bhqd,bhd->bhq", pq, z)[..., None] + 1e-6
        o = num / den
        return (lambda x, *d: x.transpose(*d))(o, 0, 2, 1, 3).reshape(B, S, D) @ wo

    def _B_ref(x, wqkv, wo):
        B, S, D = x.shape
        H = 32
        Dh = D // H
        qkv = (lambda x, *d: x.transpose(*d))((x @ wqkv).reshape(B, S, 3, H, Dh), 2, 0, 3, 1, 4)
        q, k, v = qkv[0], qkv[1], qkv[2]
        scores = jnp.einsum("bhqd,bhkd->bhqk", q, k) * (Dh ** -0.5)
        p = _softmax(scores, axis=-1)
        o = jnp.einsum("bhqk,bhkd->bhqd", p, v)
        return (lambda x, *d: x.transpose(*d))(o, 0, 2, 1, 3).reshape(B, S, D) @ wo

    x = A_x
    x = x + _A_ref(_layernorm(x, axis=-1), A_wqkv, A_wo)
    x = x + _B_ref(_layernorm(x, axis=-1), B_wqkv, B_wo)
    x = x + _A_ref(_layernorm(x, axis=-1), A_wqkv, A_wo)
    x = x + _B_ref(_layernorm(x, axis=-1), B_wqkv, B_wo)
    return x
```

```python
import functools
import math

import jax
import jax.numpy as jnp
import jax.experimental.pallas as pl
import jax.experimental.pallas.tpu as pltpu

S, D, H, DH = 2048, 1024, 32, 32
G = D // 128
NT = S // 128
TM = 256
SUB = 128
NSUB = 2
NU = G * NT
NB = NU // NSUB
W = 4 * 128
LN_EPS = 1e-5
PHI_EPS = 1e-6
QSCALE = (DH ** -0.5) * math.log2(math.e)
NT_DN = (((1,), (1,)), ((), ()))
BF16 = jnp.bfloat16
F32 = jnp.float32


def _layernorm(x):
    m = jnp.mean(x, axis=-1, keepdims=True)
    xc = x - m
    v = jnp.mean(xc * xc, axis=-1, keepdims=True)
    return (xc * jax.lax.rsqrt(v + LN_EPS)).astype(BF16)


def _phi(t):
    return jnp.where(t > 0, t + 1.0, jnp.exp(t)) + PHI_EPS


def _kernel(x_hbm, wa_hbm, woa_hbm, wb_hbm, wob_hbm, out_hbm,
            xin_ref, x_ref, wa_ref, woa_ref, wb_ref, wob_ref,
            wavt_ref, wbqt_ref, wbvt_ref,
            q_ref, k_ref, qt_ref, vt_ref, o_ref,
            kv_ref, z_ref, mm_ref, zt_ref,
            s0_ref, s1_ref, m0_ref, m1_ref, a0_ref, a1_ref, l0_ref, l1_ref,
            sems):
    cp_x = pltpu.make_async_copy(x_hbm, xin_ref, sems.at[0])
    cp_wa = pltpu.make_async_copy(wa_hbm, wa_ref, sems.at[1])
    cp_woa = pltpu.make_async_copy(woa_hbm, woa_ref, sems.at[2])
    cp_wb = pltpu.make_async_copy(wb_hbm, wb_ref, sems.at[3])
    cp_wob = pltpu.make_async_copy(wob_hbm, wob_ref, sems.at[4])
    cp_x.start()
    cp_wa.start()
    cp_woa.start()
    cp_wb.start()
    cp_wob.start()

    def transpose_w(src_ref, col0, dst_ref):
        def body(j, c):
            r0 = pl.multiple_of(j * 128, 128)
            blk = src_ref[pl.ds(r0, 128), col0:col0 + D]
            dst_ref[j] = blk.astype(F32).T.astype(BF16)
            return c
        jax.lax.fori_loop(0, D // 128, body, 0)

    def load_wt(wt_ref):
        return jnp.concatenate([wt_ref[j] for j in range(D // 128)], axis=1)

    def proj_a(xn, t):
        r0 = pl.multiple_of(t * SUB, SUB)
        qk = jnp.dot(xn, wa_ref[:, 0:2 * D], preferred_element_type=F32)
        vt = jax.lax.dot_general(load_wt(wavt_ref), xn, NT_DN,
                                 preferred_element_type=F32).astype(BF16)
        pq = _phi(qk[:, 0:D]).astype(BF16)
        pk = _phi(qk[:, D:2 * D])
        z_ref[...] += jnp.sum(pk.reshape(SUB // 8, 8, D), axis=0)
        pkb = pk.astype(BF16)
        for g in range(G):
            q_ref[g, pl.ds(r0, SUB), :] = pq[:, g * 128:(g + 1) * 128]
            kv_ref[g] += jnp.dot(vt[g * 128:(g + 1) * 128, :], pkb[:, g * 128:(g + 1) * 128],
                                 preferred_element_type=F32)

    def proj_b(xn, t):
        r0 = pl.multiple_of(t * SUB, SUB)
        k = jnp.dot(xn, wb_ref[:, D:2 * D], preferred_element_type=F32).astype(BF16)
        qt = jax.lax.dot_general(load_wt(wbqt_ref), xn, NT_DN, preferred_element_type=F32)
        qt = (qt * QSCALE).astype(BF16)
        vt = jax.lax.dot_general(load_wt(wbvt_ref), xn, NT_DN,
                                 preferred_element_type=F32).astype(BF16)
        for g in range(G):
            k_ref[g, pl.ds(r0, SUB), :] = k[:, g * 128:(g + 1) * 128]
            qt_ref[t, g] = qt[g * 128:(g + 1) * 128, :]
            vt_ref[t, g] = vt[g * 128:(g + 1) * 128, :]

    def load_rows(ref, t):
        r0 = pl.multiple_of(t * SUB, SUB)
        return jnp.concatenate([ref[g, pl.ds(r0, SUB), :] for g in range(G)], axis=1)

    def phase(src, w_ref, nxt):
        def body(i, c):
            xs = []
            for j in range(TM // SUB):
                t = i * (TM // SUB) + j
                r0 = pl.multiple_of(t * SUB, SUB)
                if src is None:
                    x = xin_ref[pl.ds(r0, SUB), :].astype(F32)
                else:
                    x = x_ref[pl.ds(r0, SUB), :] + jnp.dot(
                        load_rows(src, t), w_ref[...], preferred_element_type=F32)
                if nxt is None:
                    xin_ref[pl.ds(r0, SUB), :] = x.astype(BF16)
                else:
                    x_ref[pl.ds(r0, SUB), :] = x
                    xs.append(_layernorm(x))
            for j in range(len(xs)):
                nxt(xs[j], i * (TM // SUB) + j)
            return c
        jax.lax.fori_loop(0, S // TM, body, 0)

    def init_a():
        kv_ref[...] = jnp.zeros(kv_ref.shape, F32)
        z_ref[...] = jnp.zeros(z_ref.shape, F32)

    def mid_a():
        row_h = jax.lax.broadcasted_iota(jnp.int32, (128, 128), 0) // DH
        col_h = jax.lax.broadcasted_iota(jnp.int32, (128, 128), 1) // DH
        same = row_h == col_h
        z = jnp.sum(z_ref[...], axis=0, keepdims=True)
        for g in range(G):
            kv = jnp.where(same, kv_ref[g], 0.0).T.astype(BF16)
            mm_ref[g * 128:(g + 1) * 128, :] = jnp.dot(
                kv, woa_ref[g * 128:(g + 1) * 128, :], preferred_element_type=F32).astype(BF16)
            zb = jnp.broadcast_to(z[:, g * 128:(g + 1) * 128], (128, 128))
            zt_ref[g] = jnp.where(same, zb, 0.0).astype(BF16)

        def body(i, c):
            r0 = pl.multiple_of(i * 512, 512)
            for g in range(G):
                pq = q_ref[g, pl.ds(r0, 512), :]
                den = jax.lax.dot_general(pq, zt_ref[g], NT_DN, preferred_element_type=F32)
                o_ref[g, pl.ds(r0, 512), :] = (pq.astype(F32) / (den + PHI_EPS)).astype(BF16)
            return c
        jax.lax.fori_loop(0, S // 512, body, 0)

    def load_qm(u):
        g = u // NT
        t = u % NT
        qv = qt_ref[t, g]
        zero = jnp.zeros((DH, 128), BF16)
        cols = []
        for h in range(4):
            cols.append(jnp.concatenate(
                [qv[DH * h:DH * (h + 1)] if hh == h else zero for hh in range(4)], axis=0))
        return jnp.concatenate(cols, axis=1)

    def stage_a(u, s_ref, j, c, qm, mcur):
        g = u // NT
        kc = k_ref[g, c * 128:(c + 1) * 128, :]
        s = jnp.dot(kc, qm, preferred_element_type=F32)
        s_ref[j, c * 128:(c + 1) * 128, :] = s
        for r in range(16):
            blk = s[r * 8:(r + 1) * 8, :]
            mcur = blk if mcur is None else jnp.maximum(mcur, blk)
        return mcur

    def stage_b(u, s_ref, j, c, ms, accs, ls):
        g = u // NT
        naccs, nls = [], []
        for h in range(4):
            s = s_ref[j, c * 128:(c + 1) * 128, h * 128:(h + 1) * 128]
            p = jnp.exp2(s.reshape(16, 8, 128) - ms[h][None]).reshape(128, 128)
            l = None if ls is None else ls[h]
            for jj in range(7, -1, -1):
                r = 2 * jj
                pr = p[r * 8:(r + 1) * 8, :] + p[(r + 1) * 8:(r + 2) * 8, :]
                l = pr if l is None else l + pr
            vt = vt_ref[c, g, h * DH:(h + 1) * DH, :]
            o = jnp.dot(vt, p.astype(BF16), preferred_element_type=F32)
            naccs.append(o if accs is None else accs[h] + o)
            nls.append(l)
        return naccs, nls

    def stage_c(u, a_ref, l_ref, j):
        g = u // NT
        t = u % NT
        outs = []
        for h in range(4):
            l = jnp.sum(l_ref[j, h], axis=0, keepdims=True)
            outs.append(a_ref[j, h * DH:(h + 1) * DH, :] * (1.0 / l))
        ot = jnp.concatenate(outs, axis=0)
        o_ref[g, pl.ds(pl.multiple_of(t * 128, 128), 128), :] = ot.T.astype(BF16)

    def att_block(b, do_a, do_b, do_c, sB, mB, sA, mA, aB, lB, aC, lC):
        for j in range(NSUB):
            u = b * NSUB + j
            if do_c:
                stage_c(u - NSUB, aC, lC, j)
            if do_a:
                qm = load_qm(u + NSUB)
            if do_b:
                mm = jnp.broadcast_to(jnp.max(mB[j], axis=0, keepdims=True), (8, W))
                ms = [mm[:, h * 128:(h + 1) * 128] for h in range(4)]
            mcur = None
            accs = None
            ls = None
            for c in range(NT):
                if do_a:
                    mcur = stage_a(u + NSUB, sA, j, c, qm, mcur)
                if do_b:
                    accs, ls = stage_b(u, sB, j, c, ms, accs, ls)
            if do_a:
                mA[j] = mcur
            if do_b:
                for h in range(4):
                    aB[j, h * DH:(h + 1) * DH, :] = accs[h]
                    lB[j, h] = ls[h]

    def attention():
        bufs0 = (s0_ref, m0_ref, s1_ref, m1_ref, a0_ref, l0_ref, a1_ref, l1_ref)
        bufs1 = (s1_ref, m1_ref, s0_ref, m0_ref, a1_ref, l1_ref, a0_ref, l0_ref)
        att_block(-1, True, False, False, *bufs1)
        att_block(0, True, True, False, *bufs0)

        def body(b, c):
            @pl.when(b % 2 == 0)
            def _():
                att_block(b, True, True, True, *bufs0)

            @pl.when(b % 2 == 1)
            def _():
                att_block(b, True, True, True, *bufs1)
            return c
        jax.lax.fori_loop(1, NB - 1, body, 0)
        att_block(NB - 1, False, True, True, *bufs1)
        att_block(NB, False, False, True, *bufs0)

    cp_wa.wait()
    transpose_w(wa_ref, 2 * D, wavt_ref)
    cp_x.wait()
    init_a()
    phase(None, None, proj_a)
    cp_woa.wait()
    cp_wb.wait()
    cp_wob.wait()
    transpose_w(wb_ref, 0, wbqt_ref)
    transpose_w(wb_ref, 2 * D, wbvt_ref)

    def rep_body(rep, c):
        mid_a()
        phase(o_ref, mm_ref, proj_b)
        attention()

        @pl.when(rep == 0)
        def _():
            init_a()
            phase(o_ref, wob_ref, proj_a)
        return c
    jax.lax.fori_loop(0, 2, rep_body, 0)
    phase(o_ref, wob_ref, None)
    cp_out = pltpu.make_async_copy(xin_ref, out_hbm, sems.at[5])
    cp_out.start()
    cp_out.wait()


@jax.jit
def pallas_interleave_layers__linear_attn_block__mha_block__prompt_kernel(
    A_x: jax.Array,
    A_wqkv: jax.Array,
    A_wo: jax.Array,
    B_x: jax.Array,
    B_wqkv: jax.Array,
    B_wo: jax.Array,
):
    del B_x
    x = A_x.reshape(S, D)
    scratch = [
        pltpu.VMEM((S, D), BF16),
        pltpu.VMEM((S, D), F32),
        pltpu.VMEM((D, 3 * D), BF16),
        pltpu.VMEM((D, D), BF16),
        pltpu.VMEM((D, 3 * D), BF16),
        pltpu.VMEM((D, D), BF16),
        pltpu.VMEM((D // 128, D, 128), BF16),
        pltpu.VMEM((D // 128, D, 128), BF16),
        pltpu.VMEM((D // 128, D, 128), BF16),
        pltpu.VMEM((G, S, 128), BF16),
        pltpu.VMEM((G, S, 128), BF16),
        pltpu.VMEM((NT, G, 128, 128), BF16),
        pltpu.VMEM((NT, G, 128, 128), BF16),
        pltpu.VMEM((G, S, 128), BF16),
        pltpu.VMEM((G, 128, 128), F32),
        pltpu.VMEM((8, D), F32),
        pltpu.VMEM((D, D), BF16),
        pltpu.VMEM((G, 128, 128), BF16),
        pltpu.VMEM((NSUB, S, W), F32),
        pltpu.VMEM((NSUB, S, W), F32),
        pltpu.VMEM((NSUB, 8, W), F32),
        pltpu.VMEM((NSUB, 8, W), F32),
        pltpu.VMEM((NSUB, 128, 128), F32),
        pltpu.VMEM((NSUB, 128, 128), F32),
        pltpu.VMEM((NSUB, 4, 8, 128), F32),
        pltpu.VMEM((NSUB, 4, 8, 128), F32),
        pltpu.SemaphoreType.DMA((6,)),
    ]
    out = pl.pallas_call(
        _kernel,
        out_shape=jax.ShapeDtypeStruct((S, D), BF16),
        in_specs=[pl.BlockSpec(memory_space=pl.ANY)] * 5,
        out_specs=pl.BlockSpec(memory_space=pl.ANY),
        scratch_shapes=scratch,
        compiler_params=pltpu.CompilerParams(vmem_limit_bytes=120 * 1024 * 1024),
    )(x, A_wqkv, A_wo, B_wqkv, B_wo)
    return out.reshape(1, S, D)
```

```python
import math

import jax
import jax.numpy as jnp
import jax.experimental.pallas as pl
import jax.experimental.pallas.tpu as pltpu

S, D, H, DH = 2048, 1024, 32, 32
G = D // 128
NT = S // 128
TM = 256
T1 = 256
SUB = 128
NSUB = 4
NU = G * NT
NB = NU // NSUB
W = 4 * 128
QS = 768
LNS = 16
PC = 128
LN_EPS = 1e-5
PHI_EPS = 1e-6
QSCALE = (DH ** -0.5) * math.log2(math.e)
NT_DN = (((1,), (1,)), ((), ()))
BF16 = jnp.bfloat16
F32 = jnp.float32
SKIP = ()
MB5 = 4
MERGE = 1


def _layernorm(x):
    m = jnp.mean(x, axis=-1, keepdims=True)
    xc = x - m
    v = jnp.mean(xc * xc, axis=-1, keepdims=True)
    return (xc * jax.lax.rsqrt(v + LN_EPS)).astype(BF16)


def _phi(t):
    return jnp.where(t > 0, t + 1.0, jnp.exp(t)) + PHI_EPS


def _recip(x):
    r = pl.reciprocal(x, approx=True)
    return r * (2.0 - x * r)


def _run(gen):
    for _ in gen:
        pass


def _interleave(main, side, ratio):
    side_done = False
    for _ in main:
        for _ in range(ratio):
            if not side_done and next(side, "end") == "end":
                side_done = True
    if not side_done:
        _run(side)


def _kernel(x_hbm, wa_hbm, woa_hbm, wb_hbm, wob_hbm, out_hbm,
            xin_ref, x_ref, wa_ref, woa_ref, wb_ref, wob_ref,
            q_ref, qt_ref, vt_ref, o_ref,
            kv_ref, z_ref, mm_ref,
            s0_ref, s1_ref, m0_ref, m1_ref, a0_ref, a1_ref, l0_ref, l1_ref,
            xn_ref, sems, xsems):
    k_ref = q_ref

    def x_copy(i):
        r0 = pl.multiple_of(i * T1, T1)
        return pltpu.make_async_copy(x_hbm.at[pl.ds(r0, T1)], xin_ref.at[pl.ds(r0, T1)], xsems.at[i])

    cp_waq = pltpu.make_async_copy(wa_hbm.at[:, 0:QS], wa_ref.at[:, 0:QS], sems.at[0])
    cp_wakv = pltpu.make_async_copy(wa_hbm.at[:, QS:3 * D], wa_ref.at[:, QS:3 * D], sems.at[1])
    cp_woa = pltpu.make_async_copy(woa_hbm, woa_ref, sems.at[2])
    cp_wb = pltpu.make_async_copy(wb_hbm, wb_ref, sems.at[3])
    cp_wob = pltpu.make_async_copy(wob_hbm, wob_ref, sems.at[4])
    x_copy(0).start()
    cp_waq.start()

    def rows(t):
        if isinstance(t, int):
            return slice(t * SUB, (t + 1) * SUB)
        return pl.ds(pl.multiple_of(t * SUB, SUB), SUB)

    def mm(lhs, w_ref, c0, c1, pc):
        outs = []
        for c in range(c0, c1, pc):
            outs.append(jnp.dot(lhs, w_ref[:, c:min(c + pc, c1)], preferred_element_type=F32))
            yield
        return outs[0] if len(outs) == 1 else jnp.concatenate(outs, axis=1)

    def proj_a(xn, t, pc, q0=0, q1=D, do_kv=True):
        if do_kv:
            k = yield from mm(xn, wa_ref, D, 2 * D, pc)
            v = yield from mm(xn, wa_ref, 2 * D, 3 * D, pc)
            v = v.astype(BF16)
        q = yield from mm(xn, wa_ref, q0, q1, pc)
        pq = _phi(q).astype(BF16)
        if do_kv:
            pk = _phi(k)
            z_ref[...] += jnp.sum(pk.reshape(SUB // 8, 8, D), axis=0)
        for g in range(G):
            if do_kv:
                pkt = pk[:, g * 128:(g + 1) * 128].T.astype(BF16)
                kv_ref[g] += jnp.dot(pkt, v[:, g * 128:(g + 1) * 128], preferred_element_type=F32)
            if q0 <= g * 128 < q1:
                q_ref[g, rows(t), :] = pq[:, g * 128 - q0:(g + 1) * 128 - q0]

    def proj_b(xn, t, pc):
        q = yield from mm(xn, wb_ref, 0, D, pc)
        q = q * QSCALE
        v = yield from mm(xn, wb_ref, 2 * D, 3 * D, pc)
        k = yield from mm(xn, wb_ref, D, 2 * D, pc)
        k = k.astype(BF16)
        for g in range(G):
            qt_ref[t, g] = q[:, g * 128:(g + 1) * 128].T.astype(BF16)
            vt_ref[t, g] = v[:, g * 128:(g + 1) * 128].T.astype(BF16)
            k_ref[g, rows(t), :] = k[:, g * 128:(g + 1) * 128]

    def phase1():
        nblk = S // T1

        def ln_block(i, dst, serial=True):
            tok = None
            for j in range(T1 // LNS):
                r0 = pl.multiple_of(i * T1 + j * LNS, LNS)
                x = xin_ref[pl.ds(r0, LNS), :].astype(F32)
                if tok is not None and serial:
                    x0 = jnp.where(tok == tok, x[:, 0:128], tok)
                    x = jnp.concatenate([x0, x[:, 128:]], axis=1)
                m = jnp.mean(x, axis=-1, keepdims=True)
                xc = x - m
                v = jnp.mean(xc * xc, axis=-1, keepdims=True)
                tok = xc[:, D - 128:D]
                dst[j * LNS:(j + 1) * LNS, :] = (xc * jax.lax.rsqrt(v + LN_EPS)).astype(BF16)

        x_copy(0).wait()
        x_copy(1).start()
        ln_block(0, xn_ref.at[0:T1], False)
        cp_waq.wait()
        for i in range(2, nblk):
            x_copy(i).start()
        cp_wakv.start()

        def qbody(i, c):
            @pl.when(i + 1 < nblk)
            def _():
                x_copy(i + 1).wait()
            xv = xn_ref.at[pl.ds(pl.multiple_of(i * T1, T1), 2 * T1)]
            ln_block(jnp.minimum(i + 1, nblk - 1), xv.at[T1:2 * T1])
            for j in range(T1 // SUB):
                _run(proj_a(xv[j * SUB:(j + 1) * SUB, :], i * (T1 // SUB) + j, D, 0, QS, do_kv=False))
            return c
        jax.lax.fori_loop(0, nblk, qbody, 0)
        cp_wakv.wait()
        cp_woa.start()
        cp_wb.start()
        cp_wob.start()

        def kvbody(i, c):
            for j in range(TM // SUB):
                t = i * (TM // SUB) + j
                _run(proj_a(xn_ref[rows(t), :], t, D, QS, D))
            return c
        jax.lax.fori_loop(0, S // TM, kvbody, 0)

    def out_copy(i):
        r0 = i * TM if isinstance(i, int) else pl.multiple_of(i * TM, TM)
        return pltpu.make_async_copy(xin_ref.at[pl.ds(r0, TM)], out_hbm.at[pl.ds(r0, TM)], sems.at[5])

    def phase_block(i, w_ref, nxt, first, pc):
        xs = []
        for j in range(TM // SUB):
            t = i * (TM // SUB) + j
            lhs = jnp.concatenate([o_ref[g, rows(t), :] for g in range(G)], axis=1)
            y = yield from mm(lhs, w_ref, 0, D, pc)
            res = xin_ref[rows(t), :].astype(F32) if first else x_ref[rows(t), :]
            x = res + y
            if nxt is None:
                xin_ref[rows(t), :] = x.astype(BF16)
            else:
                x_ref[rows(t), :] = x
                xs.append(_layernorm(x))
        for j in range(len(xs)):
            yield from nxt(xs[j], i * (TM // SUB) + j, pc)

    def phase(w_ref, nxt, first=False, side=None):
        start = 0
        if side is not None:
            start = MB5 if nxt is None else 1
            npieces = start * (TM // SUB) * (D // PC) * (1 if nxt is None else 4)
            ratio = -(-(NSUB * NT) // npieces)

            def main():
                for i in range(start):
                    yield from phase_block(i, w_ref, nxt, first, PC)
            _interleave(main(), side, ratio)
            if nxt is None:
                for i in range(start):
                    out_copy(i).start()

        def body(i, c):
            _run(phase_block(i, w_ref, nxt, first, D))
            if nxt is None:
                out_copy(i).start()
            return c
        jax.lax.fori_loop(start, S // TM, body, 0)

    def init_a():
        kv_ref[...] = jnp.zeros(kv_ref.shape, F32)
        z_ref[...] = jnp.zeros(z_ref.shape, F32)

    def mid_a():
        row_h = jax.lax.broadcasted_iota(jnp.int32, (128, 128), 0) // DH
        col_h = jax.lax.broadcasted_iota(jnp.int32, (128, 128), 1) // DH
        same = row_h == col_h
        z = jnp.sum(z_ref[...], axis=0, keepdims=True)
        for g in range(G):
            zb = jnp.broadcast_to(z[:, g * 128:(g + 1) * 128], (128, 128))
            zt = jnp.where(same, zb, 0.0).astype(BF16)
            pq = q_ref[g]
            den = jax.lax.dot_general(pq, zt, NT_DN, preferred_element_type=F32)
            o_ref[g] = (pq.astype(F32) * _recip(den + PHI_EPS)).astype(BF16)
            kv = jnp.where(same, kv_ref[g], 0.0).astype(BF16)
            mm_ref[g * 128:(g + 1) * 128, :] = jnp.dot(
                kv, woa_ref[g * 128:(g + 1) * 128, :], preferred_element_type=F32).astype(BF16)

    def load_qm(u):
        qv = qt_ref[u % NT, u // NT]
        zero = jnp.zeros((DH, 128), BF16)
        cols = []
        for h in range(4):
            cols.append(jnp.concatenate(
                [qv[DH * h:DH * (h + 1)] if hh == h else zero for hh in range(4)], axis=0))
        return jnp.concatenate(cols, axis=1)

    def stage_a(u, s_ref, j, c, qm, mcur):
        kc = k_ref[u // NT, c * 128:(c + 1) * 128, :]
        s = jnp.dot(kc, qm, preferred_element_type=F32)
        s_ref[j, c * 128:(c + 1) * 128, :] = s
        for r in range(16):
            blk = s[r * 8:(r + 1) * 8, :]
            mcur = blk if mcur is None else jnp.maximum(mcur, blk)
        return mcur

    def stage_b(u, s_ref, j, c, ms, accs, ls):
        g = u // NT
        naccs, nls = [], []
        for h in range(4):
            s = s_ref[j, c * 128:(c + 1) * 128, h * 128:(h + 1) * 128]
            p = jnp.exp2(s.reshape(16, 8, 128) - ms[h][None]).reshape(128, 128)
            l = None if ls is None else ls[h]
            for jj in range(7, -1, -1):
                r = 2 * jj
                pr = p[r * 8:(r + 1) * 8, :] + p[(r + 1) * 8:(r + 2) * 8, :]
                l = pr if l is None else l + pr
            vt = vt_ref[c, g, h * DH:(h + 1) * DH, :]
            o = jnp.dot(vt, p.astype(BF16), preferred_element_type=F32)
            naccs.append(o if accs is None else accs[h] + o)
            nls.append(l)
        return naccs, nls

    def finish(u, accs, ls):
        outs = []
        for h in range(4):
            l = jnp.sum(ls[h], axis=0, keepdims=True)
            outs.append(accs[h] * (1.0 / l))
        ot = jnp.concatenate(outs, axis=0)
        o_ref[u // NT, rows(u % NT), :] = ot.T.astype(BF16)

    def att_block(b, do_a, do_b, sB, mB, sA, mA, aB, lB, aC, lC):
        for j in range(NSUB):
            u = b * NSUB + j
            if do_b:
                up = u - NSUB if isinstance(u, int) else jnp.maximum(u - NSUB, 0)
                finish(up, [aC[j, h * DH:(h + 1) * DH, :] for h in range(4)], [lC[j, h] for h in range(4)])
                mx = jnp.broadcast_to(jnp.max(mB[j], axis=0, keepdims=True), (8, W))
                ms = [mx[:, h * 128:(h + 1) * 128] for h in range(4)]
            if do_a:
                qm = load_qm(u + NSUB)
            mcur = None
            accs = None
            ls = None
            for c in range(NT):
                if do_a:
                    mcur = stage_a(u + NSUB, sA, j, c, qm, mcur)
                if do_b:
                    accs, ls = stage_b(u, sB, j, c, ms, accs, ls)
                yield
            if do_a:
                mA[j] = mcur
            if do_b and do_a:
                for h in range(4):
                    aB[j, h * DH:(h + 1) * DH, :] = accs[h]
                    lB[j, h] = ls[h]
            elif do_b:
                finish(u, accs, ls)

    def attention():
        bufs0 = (s0_ref, m0_ref, s1_ref, m1_ref, a0_ref, l0_ref, a1_ref, l1_ref)
        bufs1 = (s1_ref, m1_ref, s0_ref, m0_ref, a1_ref, l1_ref, a0_ref, l0_ref)
        a1_ref[...] = jnp.zeros(a1_ref.shape, F32)
        l1_ref[...] = jnp.ones(l1_ref.shape, F32)
        _run(att_block(-1, True, False, *bufs1))

        def body(b, c):
            @pl.when(b % 2 == 0)
            def _():
                _run(att_block(b, True, True, *bufs0))

            @pl.when(b % 2 == 1)
            def _():
                _run(att_block(b, True, True, *bufs1))
            return c
        jax.lax.fori_loop(0, NB - 1, body, 0)
        tail = att_block(NB - 1, False, True, *bufs1)
        if MERGE:
            return tail
        _run(tail)
        return None

    with jax.named_scope("p1"):
        init_a()
        phase1()
    cp_woa.wait()
    cp_wb.wait()
    cp_wob.wait()

    for rep in range(1 if "rep" in SKIP else 2):
        with jax.named_scope("mid_a"):
            mid_a()
            if rep == 0:
                init_a()
        with jax.named_scope("p2"):
            phase(mm_ref, proj_b, rep == 0)
        tail = None
        if "att" not in SKIP:
            with jax.named_scope("att"):
                tail = attention()
        if rep == 0 and "rep" not in SKIP:
            with jax.named_scope("p3"):
                phase(wob_ref, proj_a, side=tail)
    with jax.named_scope("p5"):
        phase(wob_ref, None, side=tail)
    with jax.named_scope("out"):
        pltpu.make_async_copy(xin_ref, out_hbm, sems.at[5]).wait()


@jax.jit
def pallas_interleave_layers__linear_attn_block__mha_block__prompt_kernel(
    A_x: jax.Array,
    A_wqkv: jax.Array,
    A_wo: jax.Array,
    B_x: jax.Array,
    B_wqkv: jax.Array,
    B_wo: jax.Array,
):
    del B_x
    x = A_x.reshape(S, D)
    scratch = [
        pltpu.VMEM((S, D), BF16),
        pltpu.VMEM((S, D), F32),
        pltpu.VMEM((D, 3 * D), BF16),
        pltpu.VMEM((D, D), BF16),
        pltpu.VMEM((D, 3 * D), BF16),
        pltpu.VMEM((D, D), BF16),
        pltpu.VMEM((G, S, 128), BF16),
        pltpu.VMEM((NT, G, 128, 128), BF16),
        pltpu.VMEM((NT, G, 128, 128), BF16),
        pltpu.VMEM((G, S, 128), BF16),
        pltpu.VMEM((G, 128, 128), F32),
        pltpu.VMEM((8, D), F32),
        pltpu.VMEM((D, D), BF16),
        pltpu.VMEM((NSUB, S, W), F32),
        pltpu.VMEM((NSUB, S, W), F32),
        pltpu.VMEM((NSUB, 8, W), F32),
        pltpu.VMEM((NSUB, 8, W), F32),
        pltpu.VMEM((NSUB, 128, 128), F32),
        pltpu.VMEM((NSUB, 128, 128), F32),
        pltpu.VMEM((NSUB, 4, 8, 128), F32),
        pltpu.VMEM((NSUB, 4, 8, 128), F32),
        pltpu.VMEM((S + T1, D), BF16),
        pltpu.SemaphoreType.DMA((6,)),
        pltpu.SemaphoreType.DMA((S // T1,)),
    ]
    out = pl.pallas_call(
        _kernel,
        out_shape=jax.ShapeDtypeStruct((S, D), BF16),
        in_specs=[pl.BlockSpec(memory_space=pl.ANY)] * 5,
        out_specs=pl.BlockSpec(memory_space=pl.ANY),
        scratch_shapes=scratch,
        compiler_params=pltpu.CompilerParams(vmem_limit_bytes=120 * 1024 * 1024),
    )(x, A_wqkv, A_wo, B_wqkv, B_wo)
    return out.reshape(1, S, D)
```

```python
import math

import jax
import jax.numpy as jnp
import jax.experimental.pallas as pl
import jax.experimental.pallas.tpu as pltpu

S, D, H, DH = 2048, 1024, 32, 32
G = D // 128
NT = S // 128
TM = 256
T1 = 256
SUB = 128
NSUB = 4
NU = G * NT
NB = NU // NSUB
W = 4 * 128
QS = 768
LNS = 16
PC = 128
LN_EPS = 1e-5
PHI_EPS = 1e-6
QSCALE = (DH ** -0.5) * math.log2(math.e)
NT_DN = (((1,), (1,)), ((), ()))
BF16 = jnp.bfloat16
F32 = jnp.float32
U32 = jnp.uint32
HS = SUB // 2
SKIP = ()
MB5 = 4
NOFF = 4
RC = 16
PROW = 4
GCH = 2
OFFL = 1
SORD = "gn---"
NTOK = 1
MERGE = 1


CHUNK_ORDER = []
for _o in range(NOFF):
    CHUNK_ORDER += [_o] + list(range(NOFF + 3 * _o, NOFF + 3 * (_o + 1)))


def _layernorm(x):
    m = jnp.mean(x, axis=-1, keepdims=True)
    xc = x - m
    v = jnp.mean(xc * xc, axis=-1, keepdims=True)
    return (xc * jax.lax.rsqrt(v + LN_EPS)).astype(BF16)


def _phi(t):
    return jnp.where(t > 0, t + 1.0, jnp.exp(t)) + PHI_EPS


def _recip(x):
    r = pl.reciprocal(x, approx=True)
    return r * (2.0 - x * r)


def _pk(x):
    return pltpu.bitcast(x.astype(BF16), U32)


def _upk(x):
    return pltpu.bitcast(x, BF16)


def _run(gen):
    for _ in gen:
        pass


def _interleave(main, side, ratio):
    side_done = False
    for _ in main:
        for _ in range(ratio):
            if not side_done and next(side, "end") == "end":
                side_done = True
    if not side_done:
        _run(side)


def _kernel(x_hbm, wa_hbm, woa_hbm, wb_hbm, wob_hbm, out_hbm,
            xin_ref, x_ref, wa_ref, woa_ref, wb_ref, wob_ref,
            k_ref, pqt_ref, qt_ref, vt_ref, o_ref, zc_ref, kb_ref,
            kv_ref, z_ref, mm_ref,
            s_ref, m_ref, a_ref, l_ref,
            xn_ref, sems, xsems):

    def x_copy(i):
        r0 = pl.multiple_of(i * T1, T1)
        return pltpu.make_async_copy(x_hbm.at[pl.ds(r0, T1)], xin_ref.at[pl.ds(r0, T1)], xsems.at[i])

    cp_waq = pltpu.make_async_copy(wa_hbm.at[:, 3 * D - QS:3 * D], wa_ref.at[:, 3 * D - QS:3 * D], sems.at[0])
    cp_wakv = pltpu.make_async_copy(wa_hbm.at[:, 0:3 * D - QS], wa_ref.at[:, 0:3 * D - QS], sems.at[1])
    cp_woa = pltpu.make_async_copy(woa_hbm, woa_ref, sems.at[2])
    cp_wb = pltpu.make_async_copy(wb_hbm, wb_ref, sems.at[3])
    cp_wob = pltpu.make_async_copy(wob_hbm, wob_ref, sems.at[4])
    x_copy(0).start()
    cp_waq.start()

    def rows(t):
        if isinstance(t, int):
            return slice(t * SUB, (t + 1) * SUB)
        return pl.ds(pl.multiple_of(t * SUB, SUB), SUB)

    def hrows(t):
        if isinstance(t, int):
            return slice(t * HS, (t + 1) * HS)
        return pl.ds(pl.multiple_of(t * HS, HS), HS)

    def mm(lhs, w_ref, c0, c1, pc):
        outs = []
        for c in range(c0, c1, pc):
            outs.append(jnp.dot(lhs, w_ref[:, c:min(c + pc, c1)], preferred_element_type=F32))
            yield
        return outs[0] if len(outs) == 1 else jnp.concatenate(outs, axis=1)

    def proj_a(xn, t, pc, nv=D):
        k = yield from mm(xn, wa_ref, D, 2 * D, pc)
        v = yield from mm(xn, wa_ref, 2 * D, 2 * D + nv, pc)
        v = v.astype(BF16)
        q = yield from mm(xn, wa_ref, 0, D, pc)
        pq = _phi(q)
        pk = _phi(k)
        z_ref[...] += jnp.sum(pk.reshape(SUB // 8, 8, D), axis=0)
        for g in range(G):
            pkt = pk[:, g * 128:(g + 1) * 128].T.astype(BF16)
            vg = v[:, g * 128:(g + 1) * 128] if g * 128 < nv else _upk(k_ref[g, hrows(t), :])
            kv_ref[g] += jnp.dot(pkt, vg, preferred_element_type=F32)
            pqt_ref[t, g] = pq[:, g * 128:(g + 1) * 128].T.astype(BF16)

    def proj_b(xn, t, pc):
        q = yield from mm(xn, wb_ref, 0, D, pc)
        q = q * QSCALE
        v = yield from mm(xn, wb_ref, 2 * D, 3 * D, pc)
        k = yield from mm(xn, wb_ref, D, 2 * D, pc)
        k = k.astype(BF16)
        for g in range(G):
            qt_ref[t, g] = q[:, g * 128:(g + 1) * 128].T.astype(BF16).astype(F32)
            vt_ref[t, g] = _pk(v[:, g * 128:(g + 1) * 128].T)
            k_ref[g, hrows(t), :] = _pk(k[:, g * 128:(g + 1) * 128])

    def gen_keys(srcs, gch):
        kks = [k_ref[g, (c + 1) * HS - RC // 2:(c + 1) * HS, :] for g, c in srcs]
        tok = None
        for l in range(128):
            if tok is not None and l % gch == 0:
                kks = [jnp.where(tok == tok, kk, jnp.uint32(0)) for kk in kks]
            for (g, c), kk in zip(srcs, kks):
                b = jnp.broadcast_to(_upk(kk).astype(F32)[:, l:l + 1], (RC, 128))
                kb_ref[g, l, c * RC:(c + 1) * RC, :] = b
            tok = b[0:8]

    def phase1():
        nblk = S // T1

        def ln_block(i, dst, serial=True):
            tok = None
            for j in range(T1 // LNS):
                r0 = pl.multiple_of(i * T1 + j * LNS, LNS)
                x = xin_ref[pl.ds(r0, LNS), :].astype(F32)
                if tok is not None and serial:
                    x0 = jnp.where(tok == tok, x[:, 0:128], tok)
                    x = jnp.concatenate([x0, x[:, 128:]], axis=1)
                m = jnp.mean(x, axis=-1, keepdims=True)
                xc = x - m
                v = jnp.mean(xc * xc, axis=-1, keepdims=True)
                tok = xc[:, D - 128:D]
                dst[j * LNS:(j + 1) * LNS, :] = (xc * jax.lax.rsqrt(v + LN_EPS)).astype(BF16)

        x_copy(0).wait()
        x_copy(1).start()
        ln_block(0, xn_ref.at[0:T1], False)
        cp_waq.wait()
        for i in range(2, nblk):
            x_copy(i).start()
        cp_wakv.start()

        def qbody(i, c):
            @pl.when(i + 1 < nblk)
            def _():
                x_copy(i + 1).wait()
            xv = xn_ref.at[pl.ds(pl.multiple_of(i * T1, T1), 2 * T1)]
            ln_block(jnp.minimum(i + 1, nblk - 1), xv.at[T1:2 * T1])
            for j in range(T1 // SUB):
                v = jnp.dot(xv[j * SUB:(j + 1) * SUB, :], wa_ref[:, 3 * D - QS:3 * D],
                            preferred_element_type=F32).astype(BF16)
                for g in range((D - QS) // 128, G):
                    c0 = g * 128 - (D - QS)
                    k_ref[g, hrows(i * (T1 // SUB) + j), :] = _pk(v[:, c0:c0 + 128])
            return c
        jax.lax.fori_loop(0, nblk, qbody, 0)
        cp_wakv.wait()
        cp_woa.start()
        cp_wb.start()
        cp_wob.start()

        def kvbody(i, c):
            for j in range(TM // SUB):
                t = i * (TM // SUB) + j
                _run(proj_a(xn_ref[rows(t), :], t, D, D - QS))
            return c
        jax.lax.fori_loop(0, S // TM, kvbody, 0)

    def out_copy(i):
        r0 = i * TM if isinstance(i, int) else pl.multiple_of(i * TM, TM)
        return pltpu.make_async_copy(xin_ref.at[pl.ds(r0, TM)], out_hbm.at[pl.ds(r0, TM)], sems.at[5])

    def norm_q(i, dst, serial):
        tok = None
        for j in range(TM // SUB):
            t = i * (TM // SUB) + j
            for g in range(G):
                pt = pqt_ref[t, g].astype(F32)
                w = pt * zc_ref[g]
                outs = []
                for h in range(4):
                    wh = w[h * DH:(h + 1) * DH].reshape(DH // 8, 8, 128).sum(axis=0)
                    if h == 0 and tok is not None and serial:
                        wh = jnp.where(tok == tok, wh, tok)
                    den = jnp.sum(wh, axis=0, keepdims=True) + PHI_EPS
                    outs.append(pt[h * DH:(h + 1) * DH] * (1.0 / den))
                rt = jnp.concatenate(outs, axis=0).T
                tok = outs[0][0:8] if NTOK == 0 else rt[0:8]
                dst[g, j * HS:(j + 1) * HS, :] = _pk(rt)

    def phase_block(i, w_ref, nxt, first, pc):
        xs = []
        r0 = i * (TM // 2) if isinstance(i, int) else pl.multiple_of(i * (TM // 2), TM // 2)
        ov = o_ref.at[:, pl.ds(r0, TM), :]
        if nxt is proj_b:
            def side_gen():
                if OFFL:
                    ga = (i + G - 1) % G
                    gb = (i + G - 2) % G
                    gen_keys([(ga, 0), (ga, 1), (gb, 2), (gb, 3)], GCH)

            def side_norm():
                norm_q(jnp.minimum(i + 1, S // TM - 1), ov.at[:, TM // 2:TM, :], True)
            sides = {"g": side_gen, "n": side_norm, "-": lambda: None}
            for ch in SORD[0:2]:
                sides[ch]()
        for j in range(TM // SUB):
            t = i * (TM // SUB) + j
            lhs = jnp.concatenate([_upk(ov[g, j * HS:(j + 1) * HS, :]) for g in range(G)], axis=1)
            y = yield from mm(lhs, w_ref, 0, D, pc)
            res = xin_ref[rows(t), :].astype(F32) if first else x_ref[rows(t), :]
            x = res + y
            if nxt is None:
                xin_ref[rows(t), :] = x.astype(BF16)
            else:
                x_ref[rows(t), :] = x
                xs.append(_layernorm(x))
        for j in range(len(xs)):
            if nxt is proj_b:
                sides[SORD[2 + j]]()
            yield from nxt(xs[j], i * (TM // SUB) + j, pc)
        if nxt is proj_b:
            sides[SORD[4]]()

    def phase(w_ref, nxt, first=False, side=None):
        start = 0
        if side is not None:
            start = MB5 if nxt is None else 1
            npieces = start * (TM // SUB) * (D // PC) * (1 if nxt is None else 4)
            ratio = -(-(NSUB * NT) // npieces)

            def main():
                for i in range(start):
                    yield from phase_block(i, w_ref, nxt, first, PC)
            _interleave(main(), side, ratio)
            if nxt is None:
                for i in range(start):
                    out_copy(i).start()

        def body(i, c):
            _run(phase_block(i, w_ref, nxt, first, D))
            if nxt is None:
                out_copy(i).start()
            return c
        jax.lax.fori_loop(start, S // TM, body, 0)

    def init_a():
        kv_ref[...] = jnp.zeros(kv_ref.shape, F32)
        z_ref[...] = jnp.zeros(z_ref.shape, F32)

    def mid_a():
        row_h = jax.lax.broadcasted_iota(jnp.int32, (128, 128), 0) // DH
        col_h = jax.lax.broadcasted_iota(jnp.int32, (128, 128), 1) // DH
        same = row_h == col_h
        z = jnp.sum(z_ref[...], axis=0, keepdims=True)
        for g in range(G):
            zc_ref[g] = jnp.broadcast_to(z[:, g * 128:(g + 1) * 128], (128, 128)).T
            kv = jnp.where(same, kv_ref[g], 0.0).astype(BF16)
            mm_ref[g * 128:(g + 1) * 128, :] = jnp.dot(
                kv, woa_ref[g * 128:(g + 1) * 128, :], preferred_element_type=F32).astype(BF16)
        norm_q(0, o_ref.at[:, 0:TM // 2, :], False)

    def load_qm(u):
        qv = qt_ref[u % NT, u // NT].astype(BF16)
        zero = jnp.zeros((DH, 128), BF16)
        cols = []
        for h in range(4):
            cols.append(jnp.concatenate(
                [qv[DH * h:DH * (h + 1)] if hh == h else zero for hh in range(4)], axis=0))
        return jnp.concatenate(cols, axis=1)

    def stage_a(u, s_ref, j, c, qm, mcur, pin):
        nrow = 128 - RC if (OFFL and c < NOFF) else 128
        parts = [k_ref[u // NT, c * HS + r * 8:c * HS + (r + 1) * 8, :] for r in range(nrow // 16)]
        if pin is not None:
            parts[PROW] = jnp.where(pin == pin, parts[PROW], jnp.uint32(0))
        kc = _upk(jnp.concatenate(parts, axis=0))
        s = jnp.dot(kc, qm, preferred_element_type=F32)
        s_ref[j, c * 128:c * 128 + nrow, :] = s
        for r in range(nrow // 8):
            blk = s[r * 8:(r + 1) * 8, :]
            mcur = blk if mcur is None else jnp.maximum(mcur, blk)
        return mcur

    def vpu_scores(u, j, c, h):
        g = u // NT
        t = u % NT
        accs = [None] * (RC // 8)
        for d in range(DH):
            l = h * DH + d
            qrow = jnp.broadcast_to(qt_ref[t, g, l:l + 1, :], (8, 128))
            for a in range(RC // 8):
                pr = kb_ref[g, l, c * RC + a * 8:c * RC + (a + 1) * 8, :] * qrow
                accs[a] = pr if accs[a] is None else accs[a] + pr
        mx = None
        for a in range(RC // 8):
            r0 = (c + 1) * 128 - RC + a * 8
            s_ref[j, r0:r0 + 8, h * 128:(h + 1) * 128] = accs[a]
            mx = accs[a] if mx is None else jnp.maximum(mx, accs[a])
        return mx

    def stage_b(u, s_ref, j, c, ms, accs, ls):
        g = u // NT
        naccs, nls = [], []
        for h in range(4):
            s = s_ref[j, c * 128:(c + 1) * 128, h * 128:(h + 1) * 128]
            p = jnp.exp2(s.reshape(16, 8, 128) - ms[h][None]).reshape(128, 128)
            l = None if ls is None else ls[h]
            for jj in range(7, -1, -1):
                r = 2 * jj
                pr = p[r * 8:(r + 1) * 8, :] + p[(r + 1) * 8:(r + 2) * 8, :]
                l = pr if l is None else l + pr
            vt = _upk(vt_ref[c, g, h * (DH // 2):(h + 1) * (DH // 2), :])
            o = jnp.dot(vt, p.astype(BF16), preferred_element_type=F32)
            naccs.append(o if accs is None else accs[h] + o)
            nls.append(l)
        return naccs, nls

    def finish(u, accs, ls):
        outs = []
        for h in range(4):
            l = jnp.sum(ls[h], axis=0, keepdims=True)
            outs.append(accs[h] * (1.0 / l))
        ot = jnp.concatenate(outs, axis=0)
        o_ref[u // NT, hrows(u % NT), :] = _pk(ot.T)

    def att_block(b, do_a, do_b):
        pin = None
        for j in range(NSUB):
            u = b * NSUB + j
            if do_b:
                if j == 0:
                    up = u - 1 if isinstance(u, int) else jnp.maximum(u - 1, 0)
                    finish(up, [a_ref[h * DH:(h + 1) * DH, :] for h in range(4)],
                           [l_ref[h] for h in range(4)])
                mx = jnp.broadcast_to(jnp.max(m_ref[j], axis=0, keepdims=True), (8, W))
                ms = [mx[:, h * 128:(h + 1) * 128] for h in range(4)]
            if do_a:
                qm = load_qm(u + NSUB)
            mcur = None
            accs = None
            ls = None
            mv = [None] * 4
            for n, c in enumerate(CHUNK_ORDER):
                if do_b:
                    accs, ls = stage_b(u, s_ref, j, c, ms, accs, ls)
                if do_a:
                    mcur = stage_a(u + NSUB, s_ref, j, c, qm, mcur, pin)
                    if OFFL:
                        h = n % 4
                        mx = vpu_scores(u + NSUB, j, n // 4, h)
                        mv[h] = mx if mv[h] is None else jnp.maximum(mv[h], mx)
                        pin = mv[h]
                yield
            if do_a:
                if OFFL:
                    mcur = jnp.maximum(mcur, jnp.concatenate(mv, axis=1))
                m_ref[j] = mcur
            if do_b:
                if j < NSUB - 1 or not do_a:
                    finish(u, accs, ls)
                else:
                    for h in range(4):
                        a_ref[h * DH:(h + 1) * DH, :] = accs[h]
                        l_ref[h] = ls[h]

    def attention():
        a_ref[...] = jnp.zeros(a_ref.shape, F32)
        l_ref[...] = jnp.ones(l_ref.shape, F32)
        if OFFL:
            gen_keys([(G - 1, 0), (G - 1, 1), (G - 2, 2), (G - 2, 3), (G - 1, 2), (G - 1, 3)], 4)
        _run(att_block(-1, True, False))

        def body(b, c):
            _run(att_block(b, True, True))
            return c
        jax.lax.fori_loop(0, NB - 1, body, 0)
        tail = att_block(NB - 1, False, True)
        if MERGE:
            return tail
        _run(tail)
        return None

    with jax.named_scope("p1"):
        init_a()
        phase1()
    cp_woa.wait()
    cp_wb.wait()
    cp_wob.wait()

    for rep in range(1 if "rep" in SKIP else 2):
        with jax.named_scope("mid_a"):
            mid_a()
            if rep == 0:
                init_a()
        with jax.named_scope("p2"):
            phase(mm_ref, proj_b, rep == 0)
        tail = None
        if "att" not in SKIP:
            with jax.named_scope("att"):
                tail = attention()
        if rep == 0 and "rep" not in SKIP:
            with jax.named_scope("p3"):
                phase(wob_ref, proj_a, side=tail)
    with jax.named_scope("p5"):
        phase(wob_ref, None, side=tail)
    with jax.named_scope("out"):
        pltpu.make_async_copy(xin_ref, out_hbm, sems.at[5]).wait()


@jax.jit
def pallas_interleave_layers__linear_attn_block__mha_block__prompt_kernel(
    A_x: jax.Array,
    A_wqkv: jax.Array,
    A_wo: jax.Array,
    B_x: jax.Array,
    B_wqkv: jax.Array,
    B_wo: jax.Array,
):
    del B_x
    x = A_x.reshape(S, D)
    scratch = [
        pltpu.VMEM((S, D), BF16),
        pltpu.VMEM((S, D), F32),
        pltpu.VMEM((D, 3 * D), BF16),
        pltpu.VMEM((D, D), BF16),
        pltpu.VMEM((D, 3 * D), BF16),
        pltpu.VMEM((D, D), BF16),
        pltpu.VMEM((G, S // 2, 128), U32),
        pltpu.VMEM((NT, G, 128, 128), BF16),
        pltpu.VMEM((NT, G, 128, 128), F32),
        pltpu.VMEM((NT, G, 64, 128), U32),
        pltpu.VMEM((G, (S + TM) // 2, 128), U32),
        pltpu.VMEM((G, 128, 128), F32),
        pltpu.VMEM((G, 128, NOFF * RC, 128), F32),
        pltpu.VMEM((G, 128, 128), F32),
        pltpu.VMEM((8, D), F32),
        pltpu.VMEM((D, D), BF16),
        pltpu.VMEM((NSUB, S, W), F32),
        pltpu.VMEM((NSUB, 8, W), F32),
        pltpu.VMEM((128, 128), F32),
        pltpu.VMEM((4, 8, 128), F32),
        pltpu.VMEM((S + T1, D), BF16),
        pltpu.SemaphoreType.DMA((6,)),
        pltpu.SemaphoreType.DMA((S // T1,)),
    ]
    out = pl.pallas_call(
        _kernel,
        out_shape=jax.ShapeDtypeStruct((S, D), BF16),
        in_specs=[pl.BlockSpec(memory_space=pl.ANY)] * 5,
        out_specs=pl.BlockSpec(memory_space=pl.ANY),
        scratch_shapes=scratch,
        compiler_params=pltpu.CompilerParams(vmem_limit_bytes=120 * 1024 * 1024),
    )(x, A_wqkv, A_wo, B_wqkv, B_wo)
    return out.reshape(1, S, D)
```

```python
import math

import jax
import jax.numpy as jnp
import jax.experimental.pallas as pl
import jax.experimental.pallas.tpu as pltpu

S, D, H, DH = 2048, 1024, 32, 32
G = D // 128
NT = S // 128
SUB = 128
HS = SUB // 2
TM = 256
TKV = 512
NBLK = S // TM
NSUB = 4
NU = G * NT
NB = NU // NSUB
W = 4 * 128
VS = 640
LNS = 16
NOFF = 4
RC = 16
PROW = 4
GCH = 4
MB5 = 4
LN_EPS = 1e-5
PHI_EPS = 1e-6
QSCALE = (DH ** -0.5) * math.log2(math.e)
BF16 = jnp.bfloat16
F32 = jnp.float32
U32 = jnp.uint32

CHUNK_ORDER = []
for _o in range(NOFF):
    CHUNK_ORDER += [_o] + list(range(NOFF + 3 * _o, NOFF + 3 * (_o + 1)))


def _layernorm(x):
    m = jnp.mean(x, axis=-1, keepdims=True)
    xc = x - m
    v = jnp.mean(xc * xc, axis=-1, keepdims=True)
    return (xc * jax.lax.rsqrt(v + LN_EPS)).astype(BF16)


def _phi(t):
    return jnp.where(t > 0, t + 1.0, jnp.exp(t)) + PHI_EPS


def _pk(x):
    return pltpu.bitcast(x.astype(BF16), U32)


def _upk(x):
    return pltpu.bitcast(x, BF16)


def _run(gen):
    for _ in gen:
        pass


def _interleave(main, side):
    for _ in main:
        next(side, None)
    _run(side)


def _span(i, n):
    if isinstance(i, int):
        return pl.ds(i * n, n)
    return pl.ds(pl.multiple_of(i * n, n), n)


def _kernel(x_hbm, wa_hbm, woa_hbm, wb_hbm, wob_hbm, out_hbm,
            xin_ref, x_ref, wa_ref, woa_ref, wb_ref, wob_ref,
            k_ref, pqt_ref, qt_ref, vt_ref, o_ref, zc_ref, kb_ref,
            kv_ref, z_ref, mm_ref,
            s_ref, m_ref, a_ref, l_ref,
            xn_ref, sems, xsems):
    def x_copy(i):
        return pltpu.make_async_copy(x_hbm.at[_span(i, TM)], xin_ref.at[_span(i, TM)], xsems.at[i])

    def out_copy(t, n):
        sl = pl.ds(t * SUB, n * SUB)
        return pltpu.make_async_copy(xin_ref.at[sl], out_hbm.at[sl], sems.at[5])

    c_v = 3 * D - VS
    cp_wa0 = pltpu.make_async_copy(wa_hbm.at[:, c_v:3 * D], wa_ref.at[:, c_v:3 * D], sems.at[0])
    cp_wa1 = pltpu.make_async_copy(wa_hbm.at[:, 0:c_v], wa_ref.at[:, 0:c_v], sems.at[1])
    cp_woa = pltpu.make_async_copy(woa_hbm, woa_ref, sems.at[2])
    cp_wb = pltpu.make_async_copy(wb_hbm, wb_ref, sems.at[3])
    cp_wob = pltpu.make_async_copy(wob_hbm, wob_ref, sems.at[4])
    x_copy(0).start()
    cp_wa0.start()

    def mm(lhs, w_ref, c0, c1, pc):
        outs = []
        for c in range(c0, c1, pc):
            outs.append(jnp.dot(lhs, w_ref[:, c:min(c + pc, c1)], preferred_element_type=F32))
            yield
        return outs[0] if len(outs) == 1 else jnp.concatenate(outs, axis=1)

    def proj_a(xn, t, pc, nv=D):
        k = yield from mm(xn, wa_ref, D, 2 * D, pc)
        v = yield from mm(xn, wa_ref, 2 * D, 2 * D + nv, pc)
        v = v.astype(BF16)
        q = yield from mm(xn, wa_ref, 0, D, pc)
        pq = _phi(q)
        pk = _phi(k)
        z_ref[...] += jnp.sum(pk.reshape(SUB // 8, 8, D), axis=0)
        for g in range(G):
            pkt = pk[:, g * 128:(g + 1) * 128].T.astype(BF16)
            vg = v[:, g * 128:(g + 1) * 128] if g * 128 < nv else _upk(k_ref[g, _span(t, HS), :])
            kv_ref[g] += jnp.dot(pkt, vg, preferred_element_type=F32)
            pqt_ref[t, g] = pq[:, g * 128:(g + 1) * 128].T.astype(BF16)

    def proj_b(xn, t, pc):
        q = yield from mm(xn, wb_ref, 0, D, pc)
        q = q * QSCALE
        v = yield from mm(xn, wb_ref, 2 * D, 3 * D, pc)
        k = yield from mm(xn, wb_ref, D, 2 * D, pc)
        for g in range(G):
            qt_ref[t, g] = q[:, g * 128:(g + 1) * 128].T.astype(BF16).astype(F32)
            vt_ref[t, g] = _pk(v[:, g * 128:(g + 1) * 128].T)
            k_ref[g, _span(t, HS), :] = _pk(k[:, g * 128:(g + 1) * 128])

    def gen_keys(srcs):
        kks = [k_ref[g, (c + 1) * HS - RC // 2:(c + 1) * HS, :] for g, c in srcs]
        tok = None
        for l in range(128):
            if tok is not None and l % GCH == 0:
                kks = [jnp.where(tok == tok, kk, jnp.uint32(0)) for kk in kks]
            for (g, c), kk in zip(srcs, kks):
                b = jnp.broadcast_to(_upk(kk).astype(F32)[:, l:l + 1], (RC, 128))
                kb_ref[g, l, c * RC:(c + 1) * RC, :] = b
            tok = b[0:8]

    def init_a():
        kv_ref[...] = jnp.zeros(kv_ref.shape, F32)
        z_ref[...] = jnp.zeros(z_ref.shape, F32)

    def first_phase():
        def ln_block(i, dst, serial):
            tok = None
            for j in range(TM // LNS):
                x = xin_ref[_span(i * (TM // LNS) + j, LNS), :].astype(F32)
                if tok is not None and serial:
                    x0 = jnp.where(tok == tok, x[:, 0:128], tok)
                    x = jnp.concatenate([x0, x[:, 128:]], axis=1)
                m = jnp.mean(x, axis=-1, keepdims=True)
                xc = x - m
                v = jnp.mean(xc * xc, axis=-1, keepdims=True)
                tok = xc[:, D - 128:D]
                dst[j * LNS:(j + 1) * LNS, :] = (xc * jax.lax.rsqrt(v + LN_EPS)).astype(BF16)

        x_copy(0).wait()
        x_copy(1).start()
        ln_block(0, xn_ref.at[0:TM], False)
        cp_wa0.wait()
        for i in range(2, NBLK):
            x_copy(i).start()
        cp_wa1.start()

        def vbody(i, c):
            @pl.when(i + 1 < NBLK)
            def _():
                x_copy(i + 1).wait()
            xv = xn_ref.at[pl.ds(pl.multiple_of(i * TM, TM), 2 * TM)]
            ln_block(jnp.minimum(i + 1, NBLK - 1), xv.at[TM:2 * TM], True)
            for j in range(TM // SUB):
                v = jnp.dot(xv[j * SUB:(j + 1) * SUB, :], wa_ref[:, c_v:3 * D],
                            preferred_element_type=F32)
                for g in range((D - VS) // 128, G):
                    c0 = g * 128 - (D - VS)
                    k_ref[g, _span(i * (TM // SUB) + j, HS), :] = _pk(v[:, c0:c0 + 128])
            return c
        jax.lax.fori_loop(0, NBLK, vbody, 0)
        cp_wa1.wait()
        cp_woa.start()
        cp_wb.start()
        cp_wob.start()

        def kvbody(i, c):
            for j in range(TKV // SUB):
                t = i * (TKV // SUB) + j
                _run(proj_a(xn_ref[_span(t, SUB), :], t, D, D - VS))
            return c
        jax.lax.fori_loop(0, S // TKV, kvbody, 0)

    def norm_q(i, dst, serial):
        tok = None
        for j in range(TM // SUB):
            t = i * (TM // SUB) + j
            for g in range(G):
                pt = pqt_ref[t, g].astype(F32)
                w = pt * zc_ref[g]
                outs = []
                for h in range(4):
                    wh = w[h * DH:(h + 1) * DH].reshape(DH // 8, 8, 128).sum(axis=0)
                    if h == 0 and tok is not None and serial:
                        wh = jnp.where(tok == tok, wh, tok)
                    den = jnp.sum(wh, axis=0, keepdims=True) + PHI_EPS
                    outs.append(pt[h * DH:(h + 1) * DH] * (1.0 / den))
                rt = jnp.concatenate(outs, axis=0).T
                tok = rt[0:8]
                dst[g, j * HS:(j + 1) * HS, :] = _pk(rt)

    def mid_a():
        row_h = jax.lax.broadcasted_iota(jnp.int32, (128, 128), 0) // DH
        col_h = jax.lax.broadcasted_iota(jnp.int32, (128, 128), 1) // DH
        same = row_h == col_h
        z = jnp.sum(z_ref[...], axis=0, keepdims=True)
        for g in range(G):
            zc_ref[g] = jnp.broadcast_to(z[:, g * 128:(g + 1) * 128], (128, 128)).T
            kv = jnp.where(same, kv_ref[g], 0.0).astype(BF16)
            mm_ref[g * 128:(g + 1) * 128, :] = jnp.dot(
                kv, woa_ref[g * 128:(g + 1) * 128, :], preferred_element_type=F32).astype(BF16)
        norm_q(0, o_ref.at[:, 0:TM // 2, :], False)

    def phase_block(i, w_ref, nxt, first, pc):
        r0 = i * (TM // 2) if isinstance(i, int) else pl.multiple_of(i * (TM // 2), TM // 2)
        ov = o_ref.at[:, pl.ds(r0, TM), :]
        if nxt is proj_b:
            ga = (i + G - 1) % G
            gb = (i + G - 2) % G
            gen_keys([(ga, 0), (ga, 1), (gb, 2), (gb, 3)])
            norm_q(jnp.minimum(i + 1, NBLK - 1), ov.at[:, TM // 2:TM, :], True)
        xs = []
        for j in range(TM // SUB):
            t = i * (TM // SUB) + j
            lhs = jnp.concatenate([_upk(ov[g, j * HS:(j + 1) * HS, :]) for g in range(G)], axis=1)
            y = yield from mm(lhs, w_ref, 0, D, pc)
            res = xin_ref[_span(t, SUB), :].astype(F32) if first else x_ref[_span(t, SUB), :]
            x = res + y
            x_ref[_span(t, SUB), :] = x
            xs.append(_layernorm(x))
        for j in range(TM // SUB):
            yield from nxt(xs[j], i * (TM // SUB) + j, pc)

    def phase(w_ref, nxt, first=False, side=None):
        start = 0
        if side is not None:
            _interleave(phase_block(0, w_ref, nxt, first, 128), side)
            start = 1

        def body(i, c):
            _run(phase_block(i, w_ref, nxt, first, D))
            return c
        jax.lax.fori_loop(start, NBLK, body, 0)

    def last_rows(t, n, split):
        sl = pl.ds(t * SUB, n * SUB)
        lhs = jnp.concatenate([_upk(o_ref[g, pl.ds(t * HS, n * HS), :]) for g in range(G)], axis=1)
        if split:
            for c in range(0, D, 128):
                y = x_ref[sl, c:c + 128]
                for k0 in range(0, D, D // 2):
                    y = y + jnp.dot(lhs[:, k0:k0 + D // 2], wob_ref[k0:k0 + D // 2, c:c + 128],
                                    preferred_element_type=F32)
                    yield
                xin_ref[sl, c:c + 128] = y.astype(BF16)
        else:
            y = jnp.dot(lhs, wob_ref[...], preferred_element_type=F32)
            xin_ref[sl, :] = (x_ref[sl, :] + y).astype(BF16)
        out_copy(t, n).start()

    def last_phase(side):
        def main():
            for i in range(MB5):
                yield from last_rows(2 * i, 2, True)
        _interleave(main(), side)
        for i in range(MB5, NBLK - 1):
            _run(last_rows(2 * i, 2, False))
        _run(last_rows(NT - 2, 1, False))
        _run(last_rows(NT - 1, 1, False))

    def load_qm(u):
        qv = qt_ref[u % NT, u // NT].astype(BF16)
        zero = jnp.zeros((DH, 128), BF16)
        cols = []
        for h in range(4):
            cols.append(jnp.concatenate(
                [qv[DH * h:DH * (h + 1)] if hh == h else zero for hh in range(4)], axis=0))
        return jnp.concatenate(cols, axis=1)

    def stage_a(u, j, c, qm, mcur, pin):
        nrow = 128 - RC if c < NOFF else 128
        parts = [k_ref[u // NT, c * HS + r * 8:c * HS + (r + 1) * 8, :] for r in range(nrow // 16)]
        if pin is not None:
            parts[PROW] = jnp.where(pin == pin, parts[PROW], jnp.uint32(0))
        kc = _upk(jnp.concatenate(parts, axis=0))
        s = jnp.dot(kc, qm, preferred_element_type=F32)
        s_ref[j, c * 128:c * 128 + nrow, :] = s
        for r in range(nrow // 8):
            blk = s[r * 8:(r + 1) * 8, :]
            mcur = blk if mcur is None else jnp.maximum(mcur, blk)
        return mcur

    def vpu_scores(u, j, c, h):
        g = u // NT
        t = u % NT
        accs = [None] * (RC // 8)
        for d in range(DH):
            l = h * DH + d
            qrow = jnp.broadcast_to(qt_ref[t, g, l:l + 1, :], (8, 128))
            for a in range(RC // 8):
                pr = kb_ref[g, l, c * RC + a * 8:c * RC + (a + 1) * 8, :] * qrow
                accs[a] = pr if accs[a] is None else accs[a] + pr
        mx = None
        for a in range(RC // 8):
            r0 = (c + 1) * 128 - RC + a * 8
            s_ref[j, r0:r0 + 8, h * 128:(h + 1) * 128] = accs[a]
            mx = accs[a] if mx is None else jnp.maximum(mx, accs[a])
        return mx

    def stage_b(u, j, c, ms, accs, ls):
        g = u // NT
        naccs, nls = [], []
        for h in range(4):
            s = s_ref[j, c * 128:(c + 1) * 128, h * 128:(h + 1) * 128]
            p = jnp.exp2(s.reshape(16, 8, 128) - ms[h][None]).reshape(128, 128)
            l = None if ls is None else ls[h]
            for jj in range(7, -1, -1):
                r = 2 * jj
                pr = p[r * 8:(r + 1) * 8, :] + p[(r + 1) * 8:(r + 2) * 8, :]
                l = pr if l is None else l + pr
            vt = _upk(vt_ref[c, g, h * (DH // 2):(h + 1) * (DH // 2), :])
            o = jnp.dot(vt, p.astype(BF16), preferred_element_type=F32)
            naccs.append(o if accs is None else accs[h] + o)
            nls.append(l)
        return naccs, nls

    def finish(u, accs, ls):
        outs = []
        for h in range(4):
            l = jnp.sum(ls[h], axis=0, keepdims=True)
            outs.append(accs[h] * (1.0 / l))
        ot = jnp.concatenate(outs, axis=0)
        o_ref[u // NT, _span(u % NT, HS), :] = _pk(ot.T)

    def att_block(b, do_a, do_b):
        pin = None
        for j in range(NSUB):
            u = b * NSUB + j
            if do_b:
                if j == 0:
                    up = u - 1 if isinstance(u, int) else jnp.maximum(u - 1, 0)
                    finish(up, [a_ref[h * DH:(h + 1) * DH, :] for h in range(4)],
                           [l_ref[h] for h in range(4)])
                mx = jnp.broadcast_to(jnp.max(m_ref[j], axis=0, keepdims=True), (8, W))
                ms = [mx[:, h * 128:(h + 1) * 128] for h in range(4)]
            if do_a:
                qm = load_qm(u + NSUB)
            mcur = None
            accs = None
            ls = None
            mv = [None] * 4
            for n, c in enumerate(CHUNK_ORDER):
                if do_b:
                    accs, ls = stage_b(u, j, c, ms, accs, ls)
                if do_a:
                    mcur = stage_a(u + NSUB, j, c, qm, mcur, pin)
                    h = n % 4
                    mx = vpu_scores(u + NSUB, j, n // 4, h)
                    mv[h] = mx if mv[h] is None else jnp.maximum(mv[h], mx)
                    pin = mv[h]
                yield
            if do_a:
                m_ref[j] = jnp.maximum(mcur, jnp.concatenate(mv, axis=1))
            if do_b:
                if j < NSUB - 1 or not do_a:
                    finish(u, accs, ls)
                else:
                    for h in range(4):
                        a_ref[h * DH:(h + 1) * DH, :] = accs[h]
                        l_ref[h] = ls[h]

    def attention():
        a_ref[...] = jnp.zeros(a_ref.shape, F32)
        l_ref[...] = jnp.ones(l_ref.shape, F32)
        gen_keys([(G - 1, 0), (G - 1, 1), (G - 2, 2), (G - 2, 3), (G - 1, 2), (G - 1, 3)])
        _run(att_block(-1, True, False))

        def body(b, c):
            _run(att_block(b, True, True))
            return c
        jax.lax.fori_loop(0, NB - 1, body, 0)
        return att_block(NB - 1, False, True)

    init_a()
    first_phase()
    cp_woa.wait()
    cp_wb.wait()
    cp_wob.wait()

    mid_a()
    init_a()
    phase(mm_ref, proj_b, first=True)
    tail = attention()
    phase(wob_ref, proj_a, side=tail)

    mid_a()
    phase(mm_ref, proj_b)
    tail = attention()
    last_phase(tail)
    out_copy(0, NT).wait()


@jax.jit
def pallas_interleave_layers__linear_attn_block__mha_block__prompt_kernel(
    A_x: jax.Array,
    A_wqkv: jax.Array,
    A_wo: jax.Array,
    B_x: jax.Array,
    B_wqkv: jax.Array,
    B_wo: jax.Array,
):
    del B_x
    x = A_x.reshape(S, D)
    scratch = [
        pltpu.VMEM((S, D), BF16),
        pltpu.VMEM((S, D), F32),
        pltpu.VMEM((D, 3 * D), BF16),
        pltpu.VMEM((D, D), BF16),
        pltpu.VMEM((D, 3 * D), BF16),
        pltpu.VMEM((D, D), BF16),
        pltpu.VMEM((G, S // 2, 128), U32),
        pltpu.VMEM((NT, G, 128, 128), BF16),
        pltpu.VMEM((NT, G, 128, 128), F32),
        pltpu.VMEM((NT, G, 64, 128), U32),
        pltpu.VMEM((G, (S + TM) // 2, 128), U32),
        pltpu.VMEM((G, 128, 128), F32),
        pltpu.VMEM((G, 128, NOFF * RC, 128), F32),
        pltpu.VMEM((G, 128, 128), F32),
        pltpu.VMEM((8, D), F32),
        pltpu.VMEM((D, D), BF16),
        pltpu.VMEM((NSUB, S, W), F32),
        pltpu.VMEM((NSUB, 8, W), F32),
        pltpu.VMEM((128, 128), F32),
        pltpu.VMEM((4, 8, 128), F32),
        pltpu.VMEM((S + TM, D), BF16),
        pltpu.SemaphoreType.DMA((6,)),
        pltpu.SemaphoreType.DMA((NBLK,)),
    ]
    out = pl.pallas_call(
        _kernel,
        out_shape=jax.ShapeDtypeStruct((S, D), BF16),
        in_specs=[pl.BlockSpec(memory_space=pl.ANY)] * 5,
        out_specs=pl.BlockSpec(memory_space=pl.ANY),
        scratch_shapes=scratch,
        compiler_params=pltpu.CompilerParams(vmem_limit_bytes=120 * 1024 * 1024),
    )(x, A_wqkv, A_wo, B_wqkv, B_wo)
    return out.reshape(1, S, D)
```

```python
import math

import jax
import jax.numpy as jnp
import jax.experimental.pallas as pl
import jax.experimental.pallas.tpu as pltpu

S, D, H, DH = 2048, 1024, 32, 32
G = D // 128
NT = S // 128
SUB = 128
HS = SUB // 2
TM = 256
TKV = 512
NBLK = S // TM
NSUB = 4
NU = G * NT
NB = NU // NSUB
W = 4 * 128
VS = 640
LNS = 16
NOFF = 4
RC = 16
PROW = 4
GCH = 4
MB5 = 4
LN_EPS = 1e-5
PHI_EPS = 1e-6
QSCALE = (DH ** -0.5) * math.log2(math.e)
BF16 = jnp.bfloat16
F32 = jnp.float32
U32 = jnp.uint32

CHUNK_ORDER = []
for _o in range(NOFF):
    CHUNK_ORDER += [_o] + list(range(NOFF + 3 * _o, NOFF + 3 * (_o + 1)))


def _layernorm(x):
    m = jnp.mean(x, axis=-1, keepdims=True)
    xc = x - m
    v = jnp.mean(xc * xc, axis=-1, keepdims=True)
    return (xc * jax.lax.rsqrt(v + LN_EPS)).astype(BF16)


def _phi(t):
    return jnp.where(t > 0, t + 1.0, jnp.exp(t)) + PHI_EPS


def _pk(x):
    return pltpu.bitcast(x.astype(BF16), U32)


def _upk(x):
    return pltpu.bitcast(x, BF16)


def _run(gen):
    for _ in gen:
        pass


def _interleave(main, side):
    for _ in main:
        next(side, None)
    _run(side)


def _span(i, n):
    if isinstance(i, int):
        return pl.ds(i * n, n)
    return pl.ds(pl.multiple_of(i * n, n), n)


def _kernel(x_hbm, wa_hbm, woa_hbm, wb_hbm, wob_hbm, out_hbm,
            xin_ref, x_ref, wa_ref, woa_ref, wb_ref, wob_ref,
            k_ref, pqt_ref, qt_ref, vt_ref, o_ref, zc_ref, kb_ref,
            kv_ref, z_ref, mm_ref,
            s_ref, m_ref, a_ref, l_ref,
            xn_ref, sems, xsems):
    def x_copy(i):
        return pltpu.make_async_copy(x_hbm.at[_span(i, TM)], xin_ref.at[_span(i, TM)], xsems.at[i])

    def out_copy(t, n):
        sl = pl.ds(t * SUB, n * SUB)
        return pltpu.make_async_copy(xin_ref.at[sl], out_hbm.at[sl], sems.at[5])

    c_v = 3 * D - VS
    cp_wa0 = pltpu.make_async_copy(wa_hbm.at[:, c_v:3 * D], wa_ref.at[:, c_v:3 * D], sems.at[0])
    cp_wa1 = pltpu.make_async_copy(wa_hbm.at[:, 0:c_v], wa_ref.at[:, 0:c_v], sems.at[1])
    cp_woa = pltpu.make_async_copy(woa_hbm, woa_ref, sems.at[2])
    cp_wb = pltpu.make_async_copy(wb_hbm, wb_ref, sems.at[3])
    cp_wob = pltpu.make_async_copy(wob_hbm, wob_ref, sems.at[4])
    x_copy(0).start()
    cp_wa0.start()

    def mm(lhs, w_ref, c0, c1, pc):
        outs = []
        for c in range(c0, c1, pc):
            outs.append(jnp.dot(lhs, w_ref[:, c:min(c + pc, c1)], preferred_element_type=F32))
            yield
        return outs[0] if len(outs) == 1 else jnp.concatenate(outs, axis=1)

    def proj_a(xn, t, pc, nv=D):
        k = yield from mm(xn, wa_ref, D, 2 * D, pc)
        v = yield from mm(xn, wa_ref, 2 * D, 2 * D + nv, pc)
        v = v.astype(BF16)
        q = yield from mm(xn, wa_ref, 0, D, pc)
        pq = _phi(q)
        pk = _phi(k)
        z_ref[...] += jnp.sum(pk.reshape(SUB // 8, 8, D), axis=0)
        for g in range(G):
            pkt = pk[:, g * 128:(g + 1) * 128].T.astype(BF16)
            vg = v[:, g * 128:(g + 1) * 128] if g * 128 < nv else _upk(k_ref[g, _span(t, HS), :])
            kv_ref[g] += jnp.dot(pkt, vg, preferred_element_type=F32)
            pqt_ref[t, g] = pq[:, g * 128:(g + 1) * 128].T.astype(BF16)

    def proj_b(xn, t, pc):
        q = yield from mm(xn, wb_ref, 0, D, pc)
        q = q * QSCALE
        v = yield from mm(xn, wb_ref, 2 * D, 3 * D, pc)
        k = yield from mm(xn, wb_ref, D, 2 * D, pc)
        for g in range(G):
            qt_ref[t, g] = q[:, g * 128:(g + 1) * 128].T.astype(BF16).astype(F32)
            vt_ref[t, g] = _pk(v[:, g * 128:(g + 1) * 128].T)
            k_ref[g, _span(t, HS), :] = _pk(k[:, g * 128:(g + 1) * 128])

    def gen_keys(srcs):
        kks = [jnp.concatenate([k_ref[g, (cc + 1) * HS - RC // 2:(cc + 1) * HS, :]
                                for cc in (c, c + 1)], axis=0) for g, c in srcs]
        tok = None
        for l in range(128):
            if l % GCH == 0:
                if tok is not None:
                    kks = [jnp.where(tok == tok, kk, jnp.uint32(0)) for kk in kks]
                kfs = [_upk(kk).astype(F32) for kk in kks]
            for (g, c), kf in zip(srcs, kfs):
                b = jnp.broadcast_to(kf[:, l:l + 1], (2 * RC, 128))
                kb_ref[g, l, c * RC:(c + 2) * RC, :] = b
            if l % GCH == GCH - 1:
                tok = b[RC:2 * RC]

    def init_a():
        kv_ref[...] = jnp.zeros(kv_ref.shape, F32)
        z_ref[...] = jnp.zeros(z_ref.shape, F32)

    def first_phase():
        def ln_block(i, dst, serial):
            tok = None
            for j in range(TM // LNS):
                x = xin_ref[_span(i * (TM // LNS) + j, LNS), :].astype(F32)
                if tok is not None and serial:
                    x0 = jnp.where(tok == tok, x[:, 0:128], tok)
                    x = jnp.concatenate([x0, x[:, 128:]], axis=1)
                m = jnp.mean(x, axis=-1, keepdims=True)
                xc = x - m
                v = jnp.mean(xc * xc, axis=-1, keepdims=True)
                tok = xc[:, D - 128:D]
                dst[j * LNS:(j + 1) * LNS, :] = (xc * jax.lax.rsqrt(v + LN_EPS)).astype(BF16)

        x_copy(0).wait()
        x_copy(1).start()
        ln_block(0, xn_ref.at[0:TM], False)
        cp_wa0.wait()
        for i in range(2, NBLK):
            x_copy(i).start()
        cp_wa1.start()

        def vbody(i, c):
            @pl.when(i + 1 < NBLK)
            def _():
                x_copy(i + 1).wait()
            xv = xn_ref.at[pl.ds(pl.multiple_of(i * TM, TM), 2 * TM)]
            ln_block(jnp.minimum(i + 1, NBLK - 1), xv.at[TM:2 * TM], True)
            for j in range(TM // SUB):
                v = jnp.dot(xv[j * SUB:(j + 1) * SUB, :], wa_ref[:, c_v:3 * D],
                            preferred_element_type=F32)
                for g in range((D - VS) // 128, G):
                    c0 = g * 128 - (D - VS)
                    k_ref[g, _span(i * (TM // SUB) + j, HS), :] = _pk(v[:, c0:c0 + 128])
            return c
        jax.lax.fori_loop(0, NBLK, vbody, 0)
        cp_wa1.wait()
        cp_woa.start()
        cp_wb.start()
        cp_wob.start()

        def kvbody(i, c):
            for j in range(TKV // SUB):
                t = i * (TKV // SUB) + j
                _run(proj_a(xn_ref[_span(t, SUB), :], t, D, D - VS))
            return c
        jax.lax.fori_loop(0, S // TKV, kvbody, 0)

    def norm_q(i, dst, serial):
        tok = None
        for j in range(TM // SUB):
            t = i * (TM // SUB) + j
            for g in range(G):
                pt = pqt_ref[t, g].astype(F32)
                w = pt * zc_ref[g]
                outs = []
                for h in range(4):
                    wh = w[h * DH:(h + 1) * DH].reshape(DH // 8, 8, 128).sum(axis=0)
                    if h == 0 and tok is not None and serial:
                        wh = jnp.where(tok == tok, wh, tok)
                    den = jnp.sum(wh, axis=0, keepdims=True) + PHI_EPS
                    outs.append(pt[h * DH:(h + 1) * DH] * (1.0 / den))
                rt = jnp.concatenate(outs, axis=0).T
                tok = rt[0:8]
                dst[g, j * HS:(j + 1) * HS, :] = _pk(rt)

    def mid_a():
        row_h = jax.lax.broadcasted_iota(jnp.int32, (128, 128), 0) // DH
        col_h = jax.lax.broadcasted_iota(jnp.int32, (128, 128), 1) // DH
        same = row_h == col_h
        z = jnp.sum(z_ref[...], axis=0, keepdims=True)
        for g in range(G):
            zc_ref[g] = jnp.broadcast_to(z[:, g * 128:(g + 1) * 128], (128, 128)).T
            kv = jnp.where(same, kv_ref[g], 0.0).astype(BF16)
            mm_ref[g * 128:(g + 1) * 128, :] = jnp.dot(
                kv, woa_ref[g * 128:(g + 1) * 128, :], preferred_element_type=F32).astype(BF16)
        norm_q(0, o_ref.at[:, 0:TM // 2, :], False)

    def phase_block(i, w_ref, nxt, first, pc):
        r0 = i * (TM // 2) if isinstance(i, int) else pl.multiple_of(i * (TM // 2), TM // 2)
        ov = o_ref.at[:, pl.ds(r0, TM), :]
        if nxt is proj_b:
            ga = (i + G - 1) % G
            gb = (i + G - 2) % G
            gen_keys([(ga, 0), (gb, 2)])
            norm_q(jnp.minimum(i + 1, NBLK - 1), ov.at[:, TM // 2:TM, :], True)
        xs = []
        for j in range(TM // SUB):
            t = i * (TM // SUB) + j
            lhs = jnp.concatenate([_upk(ov[g, j * HS:(j + 1) * HS, :]) for g in range(G)], axis=1)
            y = yield from mm(lhs, w_ref, 0, D, pc)
            res = xin_ref[_span(t, SUB), :].astype(F32) if first else x_ref[_span(t, SUB), :]
            x = res + y
            x_ref[_span(t, SUB), :] = x
            xs.append(_layernorm(x))
        for j in range(TM // SUB):
            yield from nxt(xs[j], i * (TM // SUB) + j, pc)

    def phase(w_ref, nxt, first=False, side=None):
        start = 0
        if side is not None:
            _interleave(phase_block(0, w_ref, nxt, first, 128), side)
            start = 1

        def body(i, c):
            _run(phase_block(i, w_ref, nxt, first, D))
            return c
        jax.lax.fori_loop(start, NBLK, body, 0)

    def last_rows(t, n, split):
        sl = pl.ds(t * SUB, n * SUB)
        lhs = jnp.concatenate([_upk(o_ref[g, pl.ds(t * HS, n * HS), :]) for g in range(G)], axis=1)
        if split:
            for c in range(0, D, 128):
                y = x_ref[sl, c:c + 128]
                for k0 in range(0, D, D // 2):
                    y = y + jnp.dot(lhs[:, k0:k0 + D // 2], wob_ref[k0:k0 + D // 2, c:c + 128],
                                    preferred_element_type=F32)
                    yield
                xin_ref[sl, c:c + 128] = y.astype(BF16)
        else:
            y = jnp.dot(lhs, wob_ref[...], preferred_element_type=F32)
            xin_ref[sl, :] = (x_ref[sl, :] + y).astype(BF16)
        out_copy(t, n).start()

    def last_phase(side):
        def main():
            for i in range(MB5):
                yield from last_rows(2 * i, 2, True)
        _interleave(main(), side)
        for i in range(MB5, NBLK - 1):
            _run(last_rows(2 * i, 2, False))
        _run(last_rows(NT - 2, 1, False))
        _run(last_rows(NT - 1, 1, False))

    def unit(n):
        return n // NT, n % NT

    def load_qm(u):
        qv = qt_ref[u[1], u[0]].astype(BF16)
        zero = jnp.zeros((DH, 128), BF16)
        cols = []
        for h in range(4):
            cols.append(jnp.concatenate(
                [qv[DH * h:DH * (h + 1)] if hh == h else zero for hh in range(4)], axis=0))
        return jnp.concatenate(cols, axis=1)

    def stage_a(u, j, c, qm, mcur, pin):
        g = u[0]
        nrow = 128 - RC if c < NOFF else 128
        r0, r1 = c * HS, c * HS + nrow // 2
        if pin is None:
            kc = k_ref[g, r0:r1, :]
        else:
            rp = r0 + PROW * 8
            mid = jnp.where(pin == pin, k_ref[g, rp:rp + 8, :], jnp.uint32(0))
            kc = jnp.concatenate([k_ref[g, r0:rp, :], mid, k_ref[g, rp + 8:r1, :]], axis=0)
        s = jnp.dot(_upk(kc), qm, preferred_element_type=F32)
        s_ref[j, c * 128:c * 128 + nrow, :] = s
        mx = jnp.max(s.reshape(nrow // 8, 8, W), axis=0)
        return mx if mcur is None else jnp.maximum(mcur, mx)

    def vpu_scores(u, j, c, h):
        g, t = u
        sc = None
        for l in range(h * DH, (h + 1) * DH):
            pr = kb_ref[g, l, c * RC:(c + 1) * RC, :] * qt_ref[t, g, l:l + 1, :]
            sc = pr if sc is None else sc + pr
        s_ref[j, (c + 1) * 128 - RC:(c + 1) * 128, h * 128:(h + 1) * 128] = sc
        return jnp.max(sc.reshape(RC // 8, 8, 128), axis=0)

    def stage_b(u, j, c, ms, accs, ls):
        naccs, nls = [], []
        for h in range(4):
            s = s_ref[j, c * 128:(c + 1) * 128, h * 128:(h + 1) * 128]
            p = jnp.exp2(s.reshape(8, 2, 8, 128) - ms[h])
            pp = jnp.sum(p, axis=1).reshape(64, 128)
            l = None if ls is None else ls[h]
            for r in range(7, -1, -1):
                pr = pp[r * 8:(r + 1) * 8]
                l = pr if l is None else l + pr
            vt = _upk(vt_ref[c, u[0], h * (DH // 2):(h + 1) * (DH // 2), :])
            o = jnp.dot(vt, p.reshape(128, 128).astype(BF16), preferred_element_type=F32)
            naccs.append(o if accs is None else accs[h] + o)
            nls.append(l)
        return naccs, nls

    def finish(u, accs, ls):
        outs = []
        for h in range(4):
            l = jnp.sum(ls[h], axis=0, keepdims=True)
            outs.append(accs[h] * (1.0 / l))
        ot = jnp.concatenate(outs, axis=0)
        o_ref[u[0], _span(u[1], HS), :] = _pk(ot.T)

    def att_block(b, do_a, do_b):
        pin = None
        for j in range(NSUB):
            n0 = b * NSUB + j
            u = unit(n0)
            ua = unit(n0 + NSUB)
            if do_b:
                if j == 0:
                    up = unit(n0 - 1 if isinstance(n0, int) else jnp.maximum(n0 - 1, 0))
                    finish(up, [a_ref[h * DH:(h + 1) * DH, :] for h in range(4)],
                           [l_ref[h] for h in range(4)])
                mx = jnp.broadcast_to(jnp.max(m_ref[j], axis=0, keepdims=True), (8, W))
                ms = [mx[:, h * 128:(h + 1) * 128].reshape(1, 1, 8, 128) for h in range(4)]
            if do_a:
                qm = load_qm(ua)
            mcur = None
            accs = None
            ls = None
            mv = [None] * 4
            for n, c in enumerate(CHUNK_ORDER):
                if do_b:
                    accs, ls = stage_b(u, j, c, ms, accs, ls)
                if do_a:
                    mcur = stage_a(ua, j, c, qm, mcur, pin)
                    h = n % 4
                    mx = vpu_scores(ua, j, n // 4, h)
                    mv[h] = mx if mv[h] is None else jnp.maximum(mv[h], mx)
                    pin = mv[h]
                yield
            if do_a:
                m_ref[j] = jnp.maximum(mcur, jnp.concatenate(mv, axis=1))
            if do_b:
                if j < NSUB - 1 or not do_a:
                    finish(u, accs, ls)
                else:
                    for h in range(4):
                        a_ref[h * DH:(h + 1) * DH, :] = accs[h]
                        l_ref[h] = ls[h]

    def attention():
        a_ref[...] = jnp.zeros(a_ref.shape, F32)
        l_ref[...] = jnp.ones(l_ref.shape, F32)
        gen_keys([(G - 1, 0), (G - 2, 2), (G - 1, 2)])
        _run(att_block(-1, True, False))

        def body(b, c):
            _run(att_block(b, True, True))
            return c
        jax.lax.fori_loop(0, NB - 1, body, 0)
        return att_block(NB - 1, False, True)

    init_a()
    first_phase()
    cp_woa.wait()
    cp_wb.wait()
    cp_wob.wait()

    mid_a()
    init_a()
    phase(mm_ref, proj_b, first=True)
    tail = attention()
    phase(wob_ref, proj_a, side=tail)

    mid_a()
    phase(mm_ref, proj_b)
    tail = attention()
    last_phase(tail)
    out_copy(0, NT).wait()


@jax.jit
def pallas_interleave_layers__linear_attn_block__mha_block__prompt_kernel(
    A_x: jax.Array,
    A_wqkv: jax.Array,
    A_wo: jax.Array,
    B_x: jax.Array,
    B_wqkv: jax.Array,
    B_wo: jax.Array,
):
    del B_x
    x = A_x.reshape(S, D)
    scratch = [
        pltpu.VMEM((S, D), BF16),
        pltpu.VMEM((S, D), F32),
        pltpu.VMEM((D, 3 * D), BF16),
        pltpu.VMEM((D, D), BF16),
        pltpu.VMEM((D, 3 * D), BF16),
        pltpu.VMEM((D, D), BF16),
        pltpu.VMEM((G, S // 2, 128), U32),
        pltpu.VMEM((NT, G, 128, 128), BF16),
        pltpu.VMEM((NT, G, 128, 128), F32),
        pltpu.VMEM((NT, G, 64, 128), U32),
        pltpu.VMEM((G, (S + TM) // 2, 128), U32),
        pltpu.VMEM((G, 128, 128), F32),
        pltpu.VMEM((G, 128, NOFF * RC, 128), F32),
        pltpu.VMEM((G, 128, 128), F32),
        pltpu.VMEM((8, D), F32),
        pltpu.VMEM((D, D), BF16),
        pltpu.VMEM((NSUB, S, W), F32),
        pltpu.VMEM((NSUB, 8, W), F32),
        pltpu.VMEM((128, 128), F32),
        pltpu.VMEM((4, 8, 128), F32),
        pltpu.VMEM((S + TM, D), BF16),
        pltpu.SemaphoreType.DMA((6,)),
        pltpu.SemaphoreType.DMA((NBLK,)),
    ]
    out = pl.pallas_call(
        _kernel,
        out_shape=jax.ShapeDtypeStruct((S, D), BF16),
        in_specs=[pl.BlockSpec(memory_space=pl.ANY)] * 5,
        out_specs=pl.BlockSpec(memory_space=pl.ANY),
        scratch_shapes=scratch,
        compiler_params=pltpu.CompilerParams(vmem_limit_bytes=120 * 1024 * 1024),
    )(x, A_wqkv, A_wo, B_wqkv, B_wo)
    return out.reshape(1, S, D)
```

```python
import math

import jax
import jax.numpy as jnp
import jax.experimental.pallas as pl
import jax.experimental.pallas.tpu as pltpu

S, D, H, DH = 2048, 1024, 32, 32
G = D // 128
NT = S // 128
SUB = 128
HS = SUB // 2
TM = 256
TKV = 512
NBLK = S // TM
NSUB = 4
NU = G * NT
NB = NU // NSUB
W = 4 * 128
VS = 640
LNS = 16
NOFF = 4
RC = 16
PROW = 4
GCH = 4
MB5 = 6
LN_EPS = 1e-5
PHI_EPS = 1e-6
QSCALE = (DH ** -0.5) * math.log2(math.e)
BF16 = jnp.bfloat16
F32 = jnp.float32
U32 = jnp.uint32

CHUNK_ORDER = []
for _o in range(NOFF):
    CHUNK_ORDER += [_o] + list(range(NOFF + 3 * _o, NOFF + 3 * (_o + 1)))


def _layernorm(x):
    m = jnp.mean(x, axis=-1, keepdims=True)
    xc = x - m
    v = jnp.mean(xc * xc, axis=-1, keepdims=True)
    return (xc * jax.lax.rsqrt(v + LN_EPS)).astype(BF16)


def _phi(t):
    return jnp.where(t > 0, t + 1.0, jnp.exp(t)) + PHI_EPS


def _pk(x):
    return pltpu.bitcast(x.astype(BF16), U32)


def _upk(x):
    return pltpu.bitcast(x, BF16)


def _run(gen):
    for _ in gen:
        pass


def _interleave(main, side, num=1, den=1):
    acc = 0
    for _ in main:
        acc += num
        while acc >= den:
            acc -= den
            next(side, None)
    _run(side)


def _span(i, n):
    if isinstance(i, int):
        return pl.ds(i * n, n)
    return pl.ds(pl.multiple_of(i * n, n), n)


def _kernel(x_hbm, wa_hbm, woa_hbm, wb_hbm, wob_hbm, out_hbm,
            xin_ref, x_ref, wa_ref, woa_ref, wb_ref, wob_ref,
            k_ref, pqt_ref, qt_ref, vt_ref, o_ref, zc_ref, kb_ref,
            kv_ref, z_ref, mm_ref,
            s_ref, m_ref, a_ref, l_ref,
            xn_ref, sems, xsems):
    def x_copy(i):
        return pltpu.make_async_copy(x_hbm.at[_span(i, TM)], xin_ref.at[_span(i, TM)], xsems.at[i])

    def out_copy(t, n):
        sl = pl.ds(t * SUB, n * SUB)
        return pltpu.make_async_copy(xin_ref.at[sl], out_hbm.at[sl], sems.at[5])

    c_v = 3 * D - VS
    cp_wa0 = pltpu.make_async_copy(wa_hbm.at[:, c_v:3 * D], wa_ref.at[:, c_v:3 * D], sems.at[0])
    cp_wa1 = pltpu.make_async_copy(wa_hbm.at[:, 0:c_v], wa_ref.at[:, 0:c_v], sems.at[1])
    cp_woa = pltpu.make_async_copy(woa_hbm, woa_ref, sems.at[2])
    cp_wb = pltpu.make_async_copy(wb_hbm, wb_ref, sems.at[3])
    cp_wob = pltpu.make_async_copy(wob_hbm, wob_ref, sems.at[4])
    x_copy(0).start()
    cp_wa0.start()

    def mm(lhs, w_ref, c0, c1, pc):
        outs = []
        for c in range(c0, c1, pc):
            outs.append(jnp.dot(lhs, w_ref[:, c:min(c + pc, c1)], preferred_element_type=F32))
            yield
        return outs[0] if len(outs) == 1 else jnp.concatenate(outs, axis=1)

    def proj_a(xn, t, pc, nv=D):
        k = yield from mm(xn, wa_ref, D, 2 * D, pc)
        v = yield from mm(xn, wa_ref, 2 * D, 2 * D + nv, pc)
        v = v.astype(BF16)
        q = yield from mm(xn, wa_ref, 0, D, pc)
        pq = _phi(q)
        pk = _phi(k)
        z_ref[...] += jnp.sum(pk.reshape(SUB // 8, 8, D), axis=0)
        for g in range(G):
            pkt = pk[:, g * 128:(g + 1) * 128].T.astype(BF16)
            vg = v[:, g * 128:(g + 1) * 128] if g * 128 < nv else _upk(k_ref[g, _span(t, HS), :])
            kv_ref[g] += jnp.dot(pkt, vg, preferred_element_type=F32)
            pqt_ref[t, g] = pq[:, g * 128:(g + 1) * 128].T.astype(BF16)

    def proj_b(xn, t, pc):
        q = yield from mm(xn, wb_ref, 0, D, pc)
        q = q * QSCALE
        v = yield from mm(xn, wb_ref, 2 * D, 3 * D, pc)
        k = yield from mm(xn, wb_ref, D, 2 * D, pc)
        for g in range(G):
            qt_ref[t, g] = q[:, g * 128:(g + 1) * 128].T.astype(BF16).astype(F32)
            vt_ref[t, g] = _pk(v[:, g * 128:(g + 1) * 128].T)
            k_ref[g, _span(t, HS), :] = _pk(k[:, g * 128:(g + 1) * 128])

    def gen_keys(srcs):
        kks = [jnp.concatenate([k_ref[g, (cc + 1) * HS - RC // 2:(cc + 1) * HS, :]
                                for cc in (c, c + 1)], axis=0) for g, c in srcs]
        tok = None
        for l in range(128):
            if l % GCH == 0:
                if tok is not None:
                    kks = [jnp.where(tok == tok, kk, jnp.uint32(0)) for kk in kks]
                kfs = [_upk(kk).astype(F32) for kk in kks]
            for (g, c), kf in zip(srcs, kfs):
                b = jnp.broadcast_to(kf[:, l:l + 1], (2 * RC, 128))
                kb_ref[g, l, c * RC:(c + 2) * RC, :] = b
            if l % GCH == GCH - 1:
                tok = b[RC:2 * RC]

    def init_a():
        kv_ref[...] = jnp.zeros(kv_ref.shape, F32)
        z_ref[...] = jnp.zeros(z_ref.shape, F32)

    def first_phase():
        def ln_block(i, dst, serial):
            tok = None
            for j in range(TM // LNS):
                x = xin_ref[_span(i * (TM // LNS) + j, LNS), :].astype(F32)
                if tok is not None and serial:
                    x0 = jnp.where(tok == tok, x[:, 0:128], tok)
                    x = jnp.concatenate([x0, x[:, 128:]], axis=1)
                m = jnp.mean(x, axis=-1, keepdims=True)
                xc = x - m
                v = jnp.mean(xc * xc, axis=-1, keepdims=True)
                tok = xc[:, D - 128:D]
                dst[j * LNS:(j + 1) * LNS, :] = (xc * jax.lax.rsqrt(v + LN_EPS)).astype(BF16)

        x_copy(0).wait()
        x_copy(1).start()
        ln_block(0, xn_ref.at[0:TM], False)
        cp_wa0.wait()
        for i in range(2, NBLK):
            x_copy(i).start()
        cp_wa1.start()

        def vbody(i, c):
            @pl.when(i + 1 < NBLK)
            def _():
                x_copy(i + 1).wait()
            xv = xn_ref.at[pl.ds(pl.multiple_of(i * TM, TM), 2 * TM)]
            ln_block(jnp.minimum(i + 1, NBLK - 1), xv.at[TM:2 * TM], True)
            for j in range(TM // SUB):
                v = jnp.dot(xv[j * SUB:(j + 1) * SUB, :], wa_ref[:, c_v:3 * D],
                            preferred_element_type=F32)
                for g in range((D - VS) // 128, G):
                    c0 = g * 128 - (D - VS)
                    k_ref[g, _span(i * (TM // SUB) + j, HS), :] = _pk(v[:, c0:c0 + 128])
            return c
        jax.lax.fori_loop(0, NBLK, vbody, 0)
        cp_wa1.wait()
        cp_woa.start()
        cp_wb.start()
        cp_wob.start()

        def kvbody(i, c):
            for j in range(TKV // SUB):
                t = i * (TKV // SUB) + j
                _run(proj_a(xn_ref[_span(t, SUB), :], t, D, D - VS))
            return c
        jax.lax.fori_loop(0, S // TKV, kvbody, 0)

    def norm_q(i, dst, serial):
        tok = None
        for j in range(TM // SUB):
            t = i * (TM // SUB) + j
            for g in range(G):
                pt = pqt_ref[t, g].astype(F32)
                w = pt * zc_ref[g]
                outs = []
                for h in range(4):
                    wh = w[h * DH:(h + 1) * DH].reshape(DH // 8, 8, 128).sum(axis=0)
                    if h == 0 and tok is not None and serial:
                        wh = jnp.where(tok == tok, wh, tok)
                    den = jnp.sum(wh, axis=0, keepdims=True) + PHI_EPS
                    outs.append(pt[h * DH:(h + 1) * DH] * (1.0 / den))
                rt = jnp.concatenate(outs, axis=0).T
                tok = rt[0:8]
                dst[g, j * HS:(j + 1) * HS, :] = _pk(rt)

    def mid_a():
        row_h = jax.lax.broadcasted_iota(jnp.int32, (128, 128), 0) // DH
        col_h = jax.lax.broadcasted_iota(jnp.int32, (128, 128), 1) // DH
        same = row_h == col_h
        z = jnp.sum(z_ref[...], axis=0, keepdims=True)
        for g in range(G):
            zc_ref[g] = jnp.broadcast_to(z[:, g * 128:(g + 1) * 128], (128, 128)).T
            kv = jnp.where(same, kv_ref[g], 0.0).astype(BF16)
            mm_ref[g * 128:(g + 1) * 128, :] = jnp.dot(
                kv, woa_ref[g * 128:(g + 1) * 128, :], preferred_element_type=F32).astype(BF16)
        norm_q(0, o_ref.at[:, 0:TM // 2, :], False)

    def phase_block(i, w_ref, nxt, first, pc):
        r0 = i * (TM // 2) if isinstance(i, int) else pl.multiple_of(i * (TM // 2), TM // 2)
        ov = o_ref.at[:, pl.ds(r0, TM), :]
        if nxt is proj_b:
            ga = (i + G - 1) % G
            gb = (i + G - 2) % G
            gen_keys([(ga, 0), (gb, 2)])
            norm_q(jnp.minimum(i + 1, NBLK - 1), ov.at[:, TM // 2:TM, :], True)
        xs = []
        for j in range(TM // SUB):
            t = i * (TM // SUB) + j
            lhs = jnp.concatenate([_upk(ov[g, j * HS:(j + 1) * HS, :]) for g in range(G)], axis=1)
            y = yield from mm(lhs, w_ref, 0, D, pc)
            res = xin_ref[_span(t, SUB), :].astype(F32) if first else x_ref[_span(t, SUB), :]
            x = res + y
            x_ref[_span(t, SUB), :] = x
            xs.append(_layernorm(x))
        for j in range(TM // SUB):
            yield from nxt(xs[j], i * (TM // SUB) + j, pc)

    def phase(w_ref, nxt, first=False, side=None):
        start = 0
        if side is not None:
            _interleave(phase_block(0, w_ref, nxt, first, 128), side)
            start = 1

        def body(i, c):
            _run(phase_block(i, w_ref, nxt, first, D))
            return c
        jax.lax.fori_loop(start, NBLK, body, 0)

    def last_rows(t, n, split):
        sl = pl.ds(t * SUB, n * SUB)
        lhs = jnp.concatenate([_upk(o_ref[g, pl.ds(t * HS, n * HS), :]) for g in range(G)], axis=1)
        if split:
            for c in range(0, D, 128):
                y = x_ref[sl, c:c + 128]
                for k0 in range(0, D, D // 2):
                    y = y + jnp.dot(lhs[:, k0:k0 + D // 2], wob_ref[k0:k0 + D // 2, c:c + 128],
                                    preferred_element_type=F32)
                    yield
                xin_ref[sl, c:c + 128] = y.astype(BF16)
        else:
            y = jnp.dot(lhs, wob_ref[...], preferred_element_type=F32)
            xin_ref[sl, :] = (x_ref[sl, :] + y).astype(BF16)
        out_copy(t, n).start()

    def last_phase(side):
        def main():
            for i in range(MB5):
                yield from last_rows(2 * i, 2, True)
        _interleave(main(), side, NSUB, MB5)
        for i in range(MB5, NBLK - 1):
            _run(last_rows(2 * i, 2, False))
        _run(last_rows(NT - 2, 1, False))
        _run(last_rows(NT - 1, 1, False))

    def unit(n):
        return n // NT, n % NT

    def load_qm(u):
        qv = qt_ref[u[1], u[0]].astype(BF16)
        zero = jnp.zeros((DH, 128), BF16)
        cols = []
        for h in range(4):
            cols.append(jnp.concatenate(
                [qv[DH * h:DH * (h + 1)] if hh == h else zero for hh in range(4)], axis=0))
        return jnp.concatenate(cols, axis=1)

    def stage_a(u, j, c, qm, mcur, pin):
        g = u[0]
        nrow = 128 - RC if c < NOFF else 128
        r0, r1 = c * HS, c * HS + nrow // 2
        if pin is None:
            kc = k_ref[g, r0:r1, :]
        else:
            rp = r0 + PROW * 8
            mid = jnp.where(pin == pin, k_ref[g, rp:rp + 8, :], jnp.uint32(0))
            kc = jnp.concatenate([k_ref[g, r0:rp, :], mid, k_ref[g, rp + 8:r1, :]], axis=0)
        s = jnp.dot(_upk(kc), qm, preferred_element_type=F32)
        s_ref[j, c * 128:c * 128 + nrow, :] = s
        mx = jnp.max(s.reshape(nrow // 8, 8, W), axis=0)
        return mx if mcur is None else jnp.maximum(mcur, mx)

    def vpu_scores(u, j, c, h):
        g, t = u
        sc = None
        for l in range(h * DH, (h + 1) * DH):
            pr = kb_ref[g, l, c * RC:(c + 1) * RC, :] * qt_ref[t, g, l:l + 1, :]
            sc = pr if sc is None else sc + pr
        s_ref[j, (c + 1) * 128 - RC:(c + 1) * 128, h * 128:(h + 1) * 128] = sc
        return jnp.max(sc.reshape(RC // 8, 8, 128), axis=0)

    def stage_b(u, j, c, ms, accs, ls):
        naccs, nls = [], []
        for h in range(4):
            s = s_ref[j, c * 128:(c + 1) * 128, h * 128:(h + 1) * 128]
            p = jnp.exp2(s.reshape(8, 2, 8, 128) - ms[h])
            pp = jnp.sum(p, axis=1).reshape(64, 128)
            l = None if ls is None else ls[h]
            for r in range(7, -1, -1):
                pr = pp[r * 8:(r + 1) * 8]
                l = pr if l is None else l + pr
            vt = _upk(vt_ref[c, u[0], h * (DH // 2):(h + 1) * (DH // 2), :])
            o = jnp.dot(vt, p.reshape(128, 128).astype(BF16), preferred_element_type=F32)
            naccs.append(o if accs is None else accs[h] + o)
            nls.append(l)
        return naccs, nls

    def finish(u, accs, ls):
        outs = []
        for h in range(4):
            l = jnp.sum(ls[h], axis=0, keepdims=True)
            outs.append(accs[h] * (1.0 / l))
        ot = jnp.concatenate(outs, axis=0)
        o_ref[u[0], _span(u[1], HS), :] = _pk(ot.T)

    def att_block(b, do_a, do_b):
        pin = None
        for j in range(NSUB):
            n0 = b * NSUB + j
            u = unit(n0)
            ua = unit(n0 + NSUB)
            if do_b:
                if j == 0:
                    up = unit(n0 - 1 if isinstance(n0, int) else jnp.maximum(n0 - 1, 0))
                    finish(up, [a_ref[h * DH:(h + 1) * DH, :] for h in range(4)],
                           [l_ref[h] for h in range(4)])
                mx = jnp.broadcast_to(jnp.max(m_ref[j], axis=0, keepdims=True), (8, W))
                ms = [mx[:, h * 128:(h + 1) * 128].reshape(1, 1, 8, 128) for h in range(4)]
            if do_a:
                qm = load_qm(ua)
            mcur = None
            accs = None
            ls = None
            mv = [None] * 4
            for n, c in enumerate(CHUNK_ORDER):
                if do_b:
                    accs, ls = stage_b(u, j, c, ms, accs, ls)
                if do_a:
                    mcur = stage_a(ua, j, c, qm, mcur, pin)
                    h = (n + 3) % 4
                    mx = vpu_scores(ua, j, n // 4, h)
                    mv[h] = mx if mv[h] is None else jnp.maximum(mv[h], mx)
                    pin = mv[h]
                yield
            if do_a:
                m_ref[j] = jnp.maximum(mcur, jnp.concatenate(mv, axis=1))
            if do_b:
                if j < NSUB - 1 or not do_a:
                    finish(u, accs, ls)
                else:
                    for h in range(4):
                        a_ref[h * DH:(h + 1) * DH, :] = accs[h]
                        l_ref[h] = ls[h]

    def attention():
        a_ref[...] = jnp.zeros(a_ref.shape, F32)
        l_ref[...] = jnp.ones(l_ref.shape, F32)
        gen_keys([(G - 1, 0), (G - 2, 2), (G - 1, 2)])
        _run(att_block(-1, True, False))

        def body(b, c):
            _run(att_block(b, True, True))
            return c
        jax.lax.fori_loop(0, NB - 1, body, 0)
        return att_block(NB - 1, False, True)

    init_a()
    first_phase()
    cp_woa.wait()
    cp_wb.wait()
    cp_wob.wait()

    mid_a()
    init_a()
    phase(mm_ref, proj_b, first=True)
    tail = attention()
    phase(wob_ref, proj_a, side=tail)

    mid_a()
    phase(mm_ref, proj_b)
    tail = attention()
    last_phase(tail)
    out_copy(0, NT).wait()


@jax.jit
def pallas_interleave_layers__linear_attn_block__mha_block__prompt_kernel(
    A_x: jax.Array,
    A_wqkv: jax.Array,
    A_wo: jax.Array,
    B_x: jax.Array,
    B_wqkv: jax.Array,
    B_wo: jax.Array,
):
    del B_x
    x = A_x.reshape(S, D)
    scratch = [
        pltpu.VMEM((S, D), BF16),
        pltpu.VMEM((S, D), F32),
        pltpu.VMEM((D, 3 * D), BF16),
        pltpu.VMEM((D, D), BF16),
        pltpu.VMEM((D, 3 * D), BF16),
        pltpu.VMEM((D, D), BF16),
        pltpu.VMEM((G, S // 2, 128), U32),
        pltpu.VMEM((NT, G, 128, 128), BF16),
        pltpu.VMEM((NT, G, 128, 128), F32),
        pltpu.VMEM((NT, G, 64, 128), U32),
        pltpu.VMEM((G, (S + TM) // 2, 128), U32),
        pltpu.VMEM((G, 128, 128), F32),
        pltpu.VMEM((G, 128, NOFF * RC, 128), F32),
        pltpu.VMEM((G, 128, 128), F32),
        pltpu.VMEM((8, D), F32),
        pltpu.VMEM((D, D), BF16),
        pltpu.VMEM((NSUB, S, W), F32),
        pltpu.VMEM((NSUB, 8, W), F32),
        pltpu.VMEM((128, 128), F32),
        pltpu.VMEM((4, 8, 128), F32),
        pltpu.VMEM((S + TM, D), BF16),
        pltpu.SemaphoreType.DMA((6,)),
        pltpu.SemaphoreType.DMA((NBLK,)),
    ]
    out = pl.pallas_call(
        _kernel,
        out_shape=jax.ShapeDtypeStruct((S, D), BF16),
        in_specs=[pl.BlockSpec(memory_space=pl.ANY)] * 5,
        out_specs=pl.BlockSpec(memory_space=pl.ANY),
        scratch_shapes=scratch,
        compiler_params=pltpu.CompilerParams(vmem_limit_bytes=120 * 1024 * 1024),
    )(x, A_wqkv, A_wo, B_wqkv, B_wo)
    return out.reshape(1, S, D)
```

```python
import math

import jax
import jax.numpy as jnp
import jax.experimental.pallas as pl
import jax.experimental.pallas.tpu as pltpu

S, D, H, DH = 2048, 1024, 32, 32
G = D // 128
NT = S // 128
SUB = 128
HS = SUB // 2
TM = 256
TKV = 512
NBLK = S // TM
NSUB = 4
NU = G * NT
NB = NU // NSUB
W = 4 * 128
VS = 640
LNS = 16
NOFF = 4
RC = 16
PROW = 4
GCH = 4
MB5 = 6
LN_EPS = 1e-5
PHI_EPS = 1e-6
QSCALE = (DH ** -0.5) * math.log2(math.e)
BF16 = jnp.bfloat16
F32 = jnp.float32
U32 = jnp.uint32

CHUNK_ORDER = []
for _o in range(NOFF):
    CHUNK_ORDER += [_o] + list(range(NOFF + 3 * _o, NOFF + 3 * (_o + 1)))


def _layernorm(x):
    m = jnp.mean(x, axis=-1, keepdims=True)
    xc = x - m
    v = jnp.mean(xc * xc, axis=-1, keepdims=True)
    return (xc * jax.lax.rsqrt(v + LN_EPS)).astype(BF16)


def _phi(t):
    return jnp.where(t > 0, t + 1.0, jnp.exp(t)) + PHI_EPS


def _pk(x):
    return pltpu.bitcast(x.astype(BF16), U32)


def _upk(x):
    return pltpu.bitcast(x, BF16)


def _run(gen):
    for _ in gen:
        pass


def _interleave(main, side, num=1, den=1):
    acc = 0
    for _ in main:
        acc += num
        while acc >= den:
            acc -= den
            next(side, None)
    _run(side)


def _span(i, n):
    if isinstance(i, int):
        return pl.ds(i * n, n)
    return pl.ds(pl.multiple_of(i * n, n), n)


def _kernel(x_hbm, wa_hbm, woa_hbm, wb_hbm, wob_hbm, out_hbm,
            xin_ref, x_ref, wa_ref, woa_ref, wb_ref, wob_ref,
            k_ref, pqt_ref, qt_ref, vt_ref, o_ref, zc_ref, kb_ref,
            kv_ref, z_ref, mm_ref,
            s_ref, m_ref, a_ref, l_ref,
            xn_ref, sems, xsems):
    def x_copy(i):
        return pltpu.make_async_copy(x_hbm.at[_span(i, TM)], xin_ref.at[_span(i, TM)], xsems.at[i])

    def out_copy(t, n):
        sl = pl.ds(t * SUB, n * SUB)
        return pltpu.make_async_copy(xin_ref.at[sl], out_hbm.at[sl], sems.at[5])

    c_v = 3 * D - VS
    cp_wa0 = pltpu.make_async_copy(wa_hbm.at[:, c_v:3 * D], wa_ref.at[:, c_v:3 * D], sems.at[0])
    cp_wa1 = pltpu.make_async_copy(wa_hbm.at[:, 0:c_v], wa_ref.at[:, 0:c_v], sems.at[1])
    cp_woa = pltpu.make_async_copy(woa_hbm, woa_ref, sems.at[2])
    cp_wb = pltpu.make_async_copy(wb_hbm, wb_ref, sems.at[3])
    cp_wob = pltpu.make_async_copy(wob_hbm, wob_ref, sems.at[4])
    x_copy(0).start()
    cp_wa0.start()

    def mm(lhs, w_ref, c0, c1, pc):
        outs = []
        for c in range(c0, c1, pc):
            outs.append(jnp.dot(lhs, w_ref[:, c:min(c + pc, c1)], preferred_element_type=F32))
            yield
        return outs[0] if len(outs) == 1 else jnp.concatenate(outs, axis=1)

    def proj_a(xn, t, pc, nv=D):
        k = yield from mm(xn, wa_ref, D, 2 * D, pc)
        v = yield from mm(xn, wa_ref, 2 * D, 2 * D + nv, pc)
        v = v.astype(BF16)
        q = yield from mm(xn, wa_ref, 0, D, pc)
        pq = _phi(q)
        pk = _phi(k)
        z_ref[...] += jnp.sum(pk.reshape(SUB // 8, 8, D), axis=0)
        for g in range(G):
            pkt = pk[:, g * 128:(g + 1) * 128].T.astype(BF16)
            vg = v[:, g * 128:(g + 1) * 128] if g * 128 < nv else _upk(k_ref[g, _span(t, HS), :])
            kv_ref[g] += jnp.dot(pkt, vg, preferred_element_type=F32)
            pqt_ref[t, g] = pq[:, g * 128:(g + 1) * 128].T.astype(BF16)

    def proj_b(xn, t, pc):
        q = yield from mm(xn, wb_ref, 0, D, pc)
        q = q * QSCALE
        v = yield from mm(xn, wb_ref, 2 * D, 3 * D, pc)
        k = yield from mm(xn, wb_ref, D, 2 * D, pc)
        for g in range(G):
            qt_ref[t, g] = q[:, g * 128:(g + 1) * 128].T.astype(BF16).astype(F32)
            vt_ref[t, g] = _pk(v[:, g * 128:(g + 1) * 128].T)
            k_ref[g, _span(t, HS), :] = _pk(k[:, g * 128:(g + 1) * 128])

    def gen_keys(srcs):
        kks = [jnp.concatenate([k_ref[g, (cc + 1) * HS - RC // 2:(cc + 1) * HS, :]
                                for cc in (c, c + 1)], axis=0) for g, c in srcs]
        tok = None
        for l in range(128):
            if l % GCH == 0:
                if tok is not None:
                    kks = [jnp.where(tok == tok, kk, jnp.uint32(0)) for kk in kks]
                kfs = [_upk(kk).astype(F32) for kk in kks]
            for (g, c), kf in zip(srcs, kfs):
                b = jnp.broadcast_to(kf[:, l:l + 1], (2 * RC, 128))
                kb_ref[g, l, c * RC:(c + 2) * RC, :] = b
            if l % GCH == GCH - 1:
                tok = b[RC:2 * RC]

    def init_a():
        kv_ref[...] = jnp.zeros(kv_ref.shape, F32)
        z_ref[...] = jnp.zeros(z_ref.shape, F32)

    def first_phase():
        def ln_block(i, dst, serial):
            tok = None
            for j in range(TM // LNS):
                x = xin_ref[_span(i * (TM // LNS) + j, LNS), :].astype(F32)
                if tok is not None and serial:
                    x0 = jnp.where(tok == tok, x[:, 0:128], tok)
                    x = jnp.concatenate([x0, x[:, 128:]], axis=1)
                m = jnp.mean(x, axis=-1, keepdims=True)
                xc = x - m
                v = jnp.mean(xc * xc, axis=-1, keepdims=True)
                tok = xc[:, D - 128:D]
                dst[j * LNS:(j + 1) * LNS, :] = (xc * jax.lax.rsqrt(v + LN_EPS)).astype(BF16)

        x_copy(0).wait()
        x_copy(1).start()
        ln_block(0, xn_ref.at[0:TM], False)
        cp_wa0.wait()
        for i in range(2, NBLK):
            x_copy(i).start()
        cp_wa1.start()

        def vbody(i, c):
            @pl.when(i + 1 < NBLK)
            def _():
                x_copy(i + 1).wait()
            xv = xn_ref.at[pl.ds(pl.multiple_of(i * TM, TM), 2 * TM)]
            ln_block(jnp.minimum(i + 1, NBLK - 1), xv.at[TM:2 * TM], True)
            for j in range(TM // SUB):
                v = jnp.dot(xv[j * SUB:(j + 1) * SUB, :], wa_ref[:, c_v:3 * D],
                            preferred_element_type=F32)
                for g in range((D - VS) // 128, G):
                    c0 = g * 128 - (D - VS)
                    k_ref[g, _span(i * (TM // SUB) + j, HS), :] = _pk(v[:, c0:c0 + 128])
            return c
        jax.lax.fori_loop(0, NBLK, vbody, 0)
        cp_wa1.wait()
        cp_woa.start()
        cp_wb.start()
        cp_wob.start()

        def kvbody(i, c):
            for j in range(TKV // SUB):
                t = i * (TKV // SUB) + j
                _run(proj_a(xn_ref[_span(t, SUB), :], t, D, D - VS))
            return c
        jax.lax.fori_loop(0, S // TKV, kvbody, 0)

    def norm_q(i, dst, serial):
        tok = None
        for j in range(TM // SUB):
            t = i * (TM // SUB) + j
            for g in range(G):
                pt = pqt_ref[t, g].astype(F32)
                w = pt * zc_ref[g]
                outs = []
                for h in range(4):
                    wh = w[h * DH:(h + 1) * DH].reshape(DH // 8, 8, 128).sum(axis=0)
                    if h == 0 and tok is not None and serial:
                        wh = jnp.where(tok == tok, wh, tok)
                    den = jnp.sum(wh, axis=0, keepdims=True) + PHI_EPS
                    outs.append(pt[h * DH:(h + 1) * DH] * (1.0 / den))
                rt = jnp.concatenate(outs, axis=0).T
                tok = rt[0:8]
                dst[g, j * HS:(j + 1) * HS, :] = _pk(rt)

    def mid_a():
        row_h = jax.lax.broadcasted_iota(jnp.int32, (128, 128), 0) // DH
        col_h = jax.lax.broadcasted_iota(jnp.int32, (128, 128), 1) // DH
        same = row_h == col_h
        z = jnp.sum(z_ref[...], axis=0, keepdims=True)
        for g in range(G):
            zc_ref[g] = jnp.broadcast_to(z[:, g * 128:(g + 1) * 128], (128, 128)).T
            kv = jnp.where(same, kv_ref[g], 0.0).astype(BF16)
            mm_ref[g * 128:(g + 1) * 128, :] = jnp.dot(
                kv, woa_ref[g * 128:(g + 1) * 128, :], preferred_element_type=F32).astype(BF16)
        norm_q(0, o_ref.at[:, 0:TM // 2, :], False)

    def phase_block(i, w_ref, nxt, first, pc):
        r0 = i * (TM // 2) if isinstance(i, int) else pl.multiple_of(i * (TM // 2), TM // 2)
        ov = o_ref.at[:, pl.ds(r0, TM), :]
        if nxt is proj_b:
            ga = (i + G - 1) % G
            gb = (i + G - 2) % G
            gen_keys([(ga, 0), (gb, 2)])
            norm_q(jnp.minimum(i + 1, NBLK - 1), ov.at[:, TM // 2:TM, :], True)
        xs = []
        for j in range(TM // SUB):
            t = i * (TM // SUB) + j
            lhs = jnp.concatenate([_upk(ov[g, j * HS:(j + 1) * HS, :]) for g in range(G)], axis=1)
            y = yield from mm(lhs, w_ref, 0, D, pc)
            res = xin_ref[_span(t, SUB), :].astype(F32) if first else x_ref[_span(t, SUB), :]
            x = res + y
            x_ref[_span(t, SUB), :] = x
            xs.append(_layernorm(x))
        for j in range(TM // SUB):
            yield from nxt(xs[j], i * (TM // SUB) + j, pc)

    def phase(w_ref, nxt, first=False, side=None):
        start = 0
        if side is not None:
            _interleave(phase_block(0, w_ref, nxt, first, 128), side)
            start = 1

        def body(i, c):
            _run(phase_block(i, w_ref, nxt, first, D))
            return c
        jax.lax.fori_loop(start, NBLK, body, 0)

    def last_rows(t, n, split):
        sl = pl.ds(t * SUB, n * SUB)
        lhs = jnp.concatenate([_upk(o_ref[g, pl.ds(t * HS, n * HS), :]) for g in range(G)], axis=1)
        if split:
            for c in range(0, D, 128):
                y = x_ref[sl, c:c + 128]
                for k0 in range(0, D, D // 2):
                    y = y + jnp.dot(lhs[:, k0:k0 + D // 2], wob_ref[k0:k0 + D // 2, c:c + 128],
                                    preferred_element_type=F32)
                    yield
                xin_ref[sl, c:c + 128] = y.astype(BF16)
        else:
            y = jnp.dot(lhs, wob_ref[...], preferred_element_type=F32)
            xin_ref[sl, :] = (x_ref[sl, :] + y).astype(BF16)
        out_copy(t, n).start()

    def last_phase(side):
        def main():
            for i in range(MB5):
                yield from last_rows(2 * i, 2, True)
        _interleave(main(), side, NSUB, MB5)
        for i in range(MB5, NBLK - 1):
            _run(last_rows(2 * i, 2, False))
        _run(last_rows(NT - 2, 1, False))
        _run(last_rows(NT - 1, 1, False))

    def unit(n):
        return n // NT, n % NT

    def load_qm(u):
        qv = qt_ref[u[1], u[0]].astype(BF16)
        zero = jnp.zeros((DH, 128), BF16)
        cols = []
        for h in range(4):
            cols.append(jnp.concatenate(
                [qv[DH * h:DH * (h + 1)] if hh == h else zero for hh in range(4)], axis=0))
        return jnp.concatenate(cols, axis=1)

    def stage_a(u, j, c, qm, mcur, pin):
        g = u[0]
        nrow = 128 - RC if c < NOFF else 128
        r0, r1 = c * HS, c * HS + nrow // 2
        if pin is None:
            kc = k_ref[g, r0:r1, :]
        else:
            rp = r0 + PROW * 8
            mid = jnp.where(pin == pin, k_ref[g, rp:rp + 8, :], jnp.uint32(0))
            kc = jnp.concatenate([k_ref[g, r0:rp, :], mid, k_ref[g, rp + 8:r1, :]], axis=0)
        s = jnp.dot(_upk(kc), qm, preferred_element_type=F32)
        s_ref[j, c * 128:c * 128 + nrow, :] = s
        mx = jnp.max(s.reshape(nrow // 8, 8, W), axis=0)
        return mx if mcur is None else jnp.maximum(mcur, mx)

    def vpu_scores(u, j, c, h):
        g, t = u
        kb = kb_ref[g, h * DH:(h + 1) * DH, c * RC:(c + 1) * RC, :].reshape(DH * RC, 128)
        qr = qt_ref[t, g, h * DH:(h + 1) * DH, :]
        sc = None
        for d in range(DH):
            pr = kb[d * RC:(d + 1) * RC] * qr[d:d + 1]
            sc = pr if sc is None else sc + pr
        s_ref[j, (c + 1) * 128 - RC:(c + 1) * 128, h * 128:(h + 1) * 128] = sc
        return jnp.max(sc.reshape(RC // 8, 8, 128), axis=0)

    def stage_b(u, j, c, ms, accs, ls):
        naccs, nls = [], []
        for h in range(4):
            s = s_ref[j, c * 128:(c + 1) * 128, h * 128:(h + 1) * 128]
            p = jnp.exp2(s.reshape(8, 2, 8, 128) - ms[h])
            pp = jnp.sum(p, axis=1).reshape(64, 128)
            l = None if ls is None else ls[h]
            for r in range(7, -1, -1):
                pr = pp[r * 8:(r + 1) * 8]
                l = pr if l is None else l + pr
            vt = _upk(vt_ref[c, u[0], h * (DH // 2):(h + 1) * (DH // 2), :])
            o = jnp.dot(vt, p.reshape(128, 128).astype(BF16), preferred_element_type=F32)
            naccs.append(o if accs is None else accs[h] + o)
            nls.append(l)
        return naccs, nls

    def finish(u, accs, ls):
        outs = []
        for h in range(4):
            l = jnp.sum(ls[h], axis=0, keepdims=True)
            outs.append(accs[h] * (1.0 / l))
        ot = jnp.concatenate(outs, axis=0)
        o_ref[u[0], _span(u[1], HS), :] = _pk(ot.T)

    def att_block(b, do_a, do_b):
        pin = None
        for j in range(NSUB):
            n0 = b * NSUB + j
            u = unit(n0)
            ua = unit(n0 + NSUB)
            if do_b:
                if j == 0:
                    up = unit(n0 - 1 if isinstance(n0, int) else jnp.maximum(n0 - 1, 0))
                    finish(up, [a_ref[h * DH:(h + 1) * DH, :] for h in range(4)],
                           [l_ref[h] for h in range(4)])
                mx = jnp.broadcast_to(jnp.max(m_ref[j], axis=0, keepdims=True), (8, W))
                ms = [mx[:, h * 128:(h + 1) * 128].reshape(1, 1, 8, 128) for h in range(4)]
            if do_a:
                qm = load_qm(ua)
            mcur = None
            accs = None
            ls = None
            mv = [None] * 4
            for n, c in enumerate(CHUNK_ORDER):
                if do_b:
                    accs, ls = stage_b(u, j, c, ms, accs, ls)
                if do_a:
                    mcur = stage_a(ua, j, c, qm, mcur, pin)
                    h = (n + 1) % 4
                    mx = vpu_scores(ua, j, n // 4, h)
                    mv[h] = mx if mv[h] is None else jnp.maximum(mv[h], mx)
                    pin = mv[h]
                yield
            if do_a:
                m_ref[j] = jnp.maximum(mcur, jnp.concatenate(mv, axis=1))
            if do_b:
                if j < NSUB - 1 or not do_a:
                    finish(u, accs, ls)
                else:
                    for h in range(4):
                        a_ref[h * DH:(h + 1) * DH, :] = accs[h]
                        l_ref[h] = ls[h]

    def attention():
        a_ref[...] = jnp.zeros(a_ref.shape, F32)
        l_ref[...] = jnp.ones(l_ref.shape, F32)
        gen_keys([(G - 1, 0), (G - 2, 2), (G - 1, 2)])
        _run(att_block(-1, True, False))

        def body(b, c):
            _run(att_block(b, True, True))
            return c
        jax.lax.fori_loop(0, NB - 1, body, 0)
        return att_block(NB - 1, False, True)

    init_a()
    first_phase()
    cp_woa.wait()
    cp_wb.wait()
    cp_wob.wait()

    mid_a()
    init_a()
    phase(mm_ref, proj_b, first=True)
    tail = attention()
    phase(wob_ref, proj_a, side=tail)

    mid_a()
    phase(mm_ref, proj_b)
    tail = attention()
    last_phase(tail)
    out_copy(0, NT).wait()


@jax.jit
def pallas_interleave_layers__linear_attn_block__mha_block__prompt_kernel(
    A_x: jax.Array,
    A_wqkv: jax.Array,
    A_wo: jax.Array,
    B_x: jax.Array,
    B_wqkv: jax.Array,
    B_wo: jax.Array,
):
    del B_x
    x = A_x.reshape(S, D)
    scratch = [
        pltpu.VMEM((S, D), BF16),
        pltpu.VMEM((S, D), F32),
        pltpu.VMEM((D, 3 * D), BF16),
        pltpu.VMEM((D, D), BF16),
        pltpu.VMEM((D, 3 * D), BF16),
        pltpu.VMEM((D, D), BF16),
        pltpu.VMEM((G, S // 2, 128), U32),
        pltpu.VMEM((NT, G, 128, 128), BF16),
        pltpu.VMEM((NT, G, 128, 128), F32),
        pltpu.VMEM((NT, G, 64, 128), U32),
        pltpu.VMEM((G, (S + TM) // 2, 128), U32),
        pltpu.VMEM((G, 128, 128), F32),
        pltpu.VMEM((G, 128, NOFF * RC, 128), F32),
        pltpu.VMEM((G, 128, 128), F32),
        pltpu.VMEM((8, D), F32),
        pltpu.VMEM((D, D), BF16),
        pltpu.VMEM((NSUB, S, W), F32),
        pltpu.VMEM((NSUB, 8, W), F32),
        pltpu.VMEM((128, 128), F32),
        pltpu.VMEM((4, 8, 128), F32),
        pltpu.VMEM((S + TM, D), BF16),
        pltpu.SemaphoreType.DMA((6,)),
        pltpu.SemaphoreType.DMA((NBLK,)),
    ]
    out = pl.pallas_call(
        _kernel,
        out_shape=jax.ShapeDtypeStruct((S, D), BF16),
        in_specs=[pl.BlockSpec(memory_space=pl.ANY)] * 5,
        out_specs=pl.BlockSpec(memory_space=pl.ANY),
        scratch_shapes=scratch,
        compiler_params=pltpu.CompilerParams(vmem_limit_bytes=120 * 1024 * 1024),
    )(x, A_wqkv, A_wo, B_wqkv, B_wo)
    return out.reshape(1, S, D)
```

```python
import math

import jax
import jax.numpy as jnp
import jax.experimental.pallas as pl
import jax.experimental.pallas.tpu as pltpu

S, D, H, DH = 2048, 1024, 32, 32
G = D // 128
NT = S // 128
SUB = 128
HS = SUB // 2
TM = 256
TKV = 512
NBLK = S // TM
NSUB = 4
NU = G * NT
NB = NU // NSUB
W = 4 * 128
VS = 640
LNS = 16
NOFF = 4
RC = 16
PROW = 4
GCH = 4
MB5 = 6
LN_EPS = 1e-5
PHI_EPS = 1e-6
QSCALE = (DH ** -0.5) * math.log2(math.e)
BF16 = jnp.bfloat16
F32 = jnp.float32
U32 = jnp.uint32

CHUNK_ORDER = []
for _o in range(NOFF):
    CHUNK_ORDER += [_o] + list(range(NOFF + 3 * _o, NOFF + 3 * (_o + 1)))


def _layernorm(x):
    m = jnp.mean(x, axis=-1, keepdims=True)
    xc = x - m
    v = jnp.mean(xc * xc, axis=-1, keepdims=True)
    return (xc * jax.lax.rsqrt(v + LN_EPS)).astype(BF16)


def _phi(t):
    return jnp.where(t > 0, t + 1.0, jnp.exp(t)) + PHI_EPS


def _pk(x):
    return pltpu.bitcast(x.astype(BF16), U32)


def _upk(x):
    return pltpu.bitcast(x, BF16)


def _run(gen):
    for _ in gen:
        pass


def _interleave(main, side, num=1, den=1):
    acc = 0
    for _ in main:
        acc += num
        while acc >= den:
            acc -= den
            next(side, None)
    _run(side)


def _span(i, n):
    if isinstance(i, int):
        return pl.ds(i * n, n)
    return pl.ds(pl.multiple_of(i * n, n), n)


def _kernel(x_hbm, wa_hbm, woa_hbm, wb_hbm, wob_hbm, out_hbm,
            xin_ref, x_ref, wa_ref, woa_ref, wb_ref, wob_ref,
            k_ref, pqt_ref, qt_ref, vt_ref, o_ref, zc_ref, kb_ref,
            kv_ref, z_ref, mm_ref,
            s_ref, m_ref, a_ref, l_ref,
            xn_ref, sems, xsems):
    def x_copy(i):
        return pltpu.make_async_copy(x_hbm.at[_span(i, TM)], xin_ref.at[_span(i, TM)], xsems.at[i])

    def out_copy(t, n):
        sl = pl.ds(t * SUB, n * SUB)
        return pltpu.make_async_copy(xin_ref.at[sl], out_hbm.at[sl], sems.at[5])

    c_v = 3 * D - VS
    cp_wa0 = pltpu.make_async_copy(wa_hbm.at[:, c_v:3 * D], wa_ref.at[:, c_v:3 * D], sems.at[0])
    cp_wa1 = pltpu.make_async_copy(wa_hbm.at[:, 0:c_v], wa_ref.at[:, 0:c_v], sems.at[1])
    cp_woa = pltpu.make_async_copy(woa_hbm, woa_ref, sems.at[2])
    cp_wb = pltpu.make_async_copy(wb_hbm, wb_ref, sems.at[3])
    cp_wob = pltpu.make_async_copy(wob_hbm, wob_ref, sems.at[4])
    x_copy(0).start()
    cp_wa0.start()

    def mm(lhs, w_ref, c0, c1, pc):
        outs = []
        for c in range(c0, c1, pc):
            outs.append(jnp.dot(lhs, w_ref[:, c:min(c + pc, c1)], preferred_element_type=F32))
            yield
        return outs[0] if len(outs) == 1 else jnp.concatenate(outs, axis=1)

    def proj_a(xn, t, pc, nv=D):
        k = yield from mm(xn, wa_ref, D, 2 * D, pc)
        v = yield from mm(xn, wa_ref, 2 * D, 2 * D + nv, pc)
        v = v.astype(BF16)
        q = yield from mm(xn, wa_ref, 0, D, pc)
        pq = _phi(q)
        pk = _phi(k)
        z_ref[...] += jnp.sum(pk.reshape(SUB // 8, 8, D), axis=0)
        for g in range(G):
            pkt = pk[:, g * 128:(g + 1) * 128].T.astype(BF16)
            vg = v[:, g * 128:(g + 1) * 128] if g * 128 < nv else _upk(k_ref[g, _span(t, HS), :])
            kv_ref[g] += jnp.dot(pkt, vg, preferred_element_type=F32)
            pqt_ref[t, g] = pq[:, g * 128:(g + 1) * 128].T.astype(BF16)

    def proj_b(xn, t, pc):
        q = yield from mm(xn, wb_ref, 0, D, pc)
        q = q * QSCALE
        v = yield from mm(xn, wb_ref, 2 * D, 3 * D, pc)
        k = yield from mm(xn, wb_ref, D, 2 * D, pc)
        for g in range(G):
            qt_ref[t, g] = q[:, g * 128:(g + 1) * 128].T.astype(BF16).astype(F32)
            vt_ref[t, g] = _pk(v[:, g * 128:(g + 1) * 128].T)
            k_ref[g, _span(t, HS), :] = _pk(k[:, g * 128:(g + 1) * 128])

    def gen_keys(srcs):
        kks = [jnp.concatenate([k_ref[g, (cc + 1) * HS - RC // 2:(cc + 1) * HS, :]
                                for cc in (c, c + 1)], axis=0) for g, c in srcs]
        tok = None
        for l in range(128):
            if l % GCH == 0:
                if tok is not None:
                    kks = [jnp.where(tok == tok, kk, jnp.uint32(0)) for kk in kks]
                kfs = [_upk(kk).astype(F32) for kk in kks]
            for (g, c), kf in zip(srcs, kfs):
                b = jnp.broadcast_to(kf[:, l:l + 1], (2 * RC, 128))
                kb_ref[g, l, c * RC:(c + 2) * RC, :] = b
            if l % GCH == GCH - 1:
                tok = b[RC:2 * RC]

    def init_a():
        kv_ref[...] = jnp.zeros(kv_ref.shape, F32)
        z_ref[...] = jnp.zeros(z_ref.shape, F32)

    def first_phase():
        def ln_block(i, dst, serial):
            tok = None
            for j in range(TM // LNS):
                x = xin_ref[_span(i * (TM // LNS) + j, LNS), :].astype(F32)
                if tok is not None and serial:
                    x0 = jnp.where(tok == tok, x[:, 0:128], tok)
                    x = jnp.concatenate([x0, x[:, 128:]], axis=1)
                m = jnp.mean(x, axis=-1, keepdims=True)
                xc = x - m
                v = jnp.mean(xc * xc, axis=-1, keepdims=True)
                tok = xc[:, D - 128:D]
                dst[j * LNS:(j + 1) * LNS, :] = (xc * jax.lax.rsqrt(v + LN_EPS)).astype(BF16)

        x_copy(0).wait()
        x_copy(1).start()
        ln_block(0, xn_ref.at[0:TM], False)
        cp_wa0.wait()
        for i in range(2, NBLK):
            x_copy(i).start()
        cp_wa1.start()

        def vbody(i, c):
            @pl.when(i + 1 < NBLK)
            def _():
                x_copy(i + 1).wait()
            xv = xn_ref.at[pl.ds(pl.multiple_of(i * TM, TM), 2 * TM)]
            ln_block(jnp.minimum(i + 1, NBLK - 1), xv.at[TM:2 * TM], True)
            for j in range(TM // SUB):
                v = jnp.dot(xv[j * SUB:(j + 1) * SUB, :], wa_ref[:, c_v:3 * D],
                            preferred_element_type=F32)
                for g in range((D - VS) // 128, G):
                    c0 = g * 128 - (D - VS)
                    k_ref[g, _span(i * (TM // SUB) + j, HS), :] = _pk(v[:, c0:c0 + 128])
            return c
        jax.lax.fori_loop(0, NBLK, vbody, 0)
        cp_wa1.wait()
        cp_woa.start()
        cp_wb.start()
        cp_wob.start()

        def kvbody(i, c):
            for j in range(TKV // SUB):
                t = i * (TKV // SUB) + j
                _run(proj_a(xn_ref[_span(t, SUB), :], t, D, D - VS))
            return c
        jax.lax.fori_loop(0, S // TKV, kvbody, 0)

    def norm_q(i, dst, serial):
        tok = None
        for j in range(TM // SUB):
            t = i * (TM // SUB) + j
            for g in range(G):
                pt = pqt_ref[t, g].astype(F32)
                w = pt * zc_ref[g]
                outs = []
                for h in range(4):
                    wh = w[h * DH:(h + 1) * DH].reshape(DH // 8, 8, 128).sum(axis=0)
                    if h == 0 and tok is not None and serial:
                        wh = jnp.where(tok == tok, wh, tok)
                    den = jnp.sum(wh, axis=0, keepdims=True) + PHI_EPS
                    outs.append(pt[h * DH:(h + 1) * DH] * (1.0 / den))
                rt = jnp.concatenate(outs, axis=0).T
                tok = rt[0:8]
                dst[g, j * HS:(j + 1) * HS, :] = _pk(rt)

    def mid_a():
        row_h = jax.lax.broadcasted_iota(jnp.int32, (128, 128), 0) // DH
        col_h = jax.lax.broadcasted_iota(jnp.int32, (128, 128), 1) // DH
        same = row_h == col_h
        z = jnp.sum(z_ref[...], axis=0, keepdims=True)
        for g in range(G):
            zc_ref[g] = jnp.broadcast_to(z[:, g * 128:(g + 1) * 128], (128, 128)).T
            kv = jnp.where(same, kv_ref[g], 0.0).astype(BF16)
            mm_ref[g * 128:(g + 1) * 128, :] = jnp.dot(
                kv, woa_ref[g * 128:(g + 1) * 128, :], preferred_element_type=F32).astype(BF16)
        norm_q(0, o_ref.at[:, 0:TM // 2, :], False)

    def phase_block(i, w_ref, nxt, first, pc):
        r0 = i * (TM // 2) if isinstance(i, int) else pl.multiple_of(i * (TM // 2), TM // 2)
        ov = o_ref.at[:, pl.ds(r0, TM), :]
        if nxt is proj_b:
            ga = (i + G - 1) % G
            gb = (i + G - 2) % G
            gen_keys([(ga, 0), (gb, 2)])
            norm_q(jnp.minimum(i + 1, NBLK - 1), ov.at[:, TM // 2:TM, :], True)
        xs = []
        for j in range(TM // SUB):
            t = i * (TM // SUB) + j
            lhs = jnp.concatenate([_upk(ov[g, j * HS:(j + 1) * HS, :]) for g in range(G)], axis=1)
            y = yield from mm(lhs, w_ref, 0, D, pc)
            res = xin_ref[_span(t, SUB), :].astype(F32) if first else x_ref[_span(t, SUB), :]
            x = res + y
            x_ref[_span(t, SUB), :] = x
            xs.append(_layernorm(x))
        for j in range(TM // SUB):
            yield from nxt(xs[j], i * (TM // SUB) + j, pc)

    def phase(w_ref, nxt, first=False, side=None):
        start = 0
        if side is not None:
            _interleave(phase_block(0, w_ref, nxt, first, 128), side)
            start = 1

        def body(i, c):
            _run(phase_block(i, w_ref, nxt, first, D))
            return c
        jax.lax.fori_loop(start, NBLK, body, 0)

    def last_rows(t, n, split):
        sl = pl.ds(t * SUB, n * SUB)
        lhs = jnp.concatenate([_upk(o_ref[g, pl.ds(t * HS, n * HS), :]) for g in range(G)], axis=1)
        if split:
            for c in range(0, D, 128):
                y = x_ref[sl, c:c + 128]
                for k0 in range(0, D, D // 2):
                    y = y + jnp.dot(lhs[:, k0:k0 + D // 2], wob_ref[k0:k0 + D // 2, c:c + 128],
                                    preferred_element_type=F32)
                    yield
                xin_ref[sl, c:c + 128] = y.astype(BF16)
        else:
            y = jnp.dot(lhs, wob_ref[...], preferred_element_type=F32)
            xin_ref[sl, :] = (x_ref[sl, :] + y).astype(BF16)
        out_copy(t, n).start()

    def last_phase(side):
        def main():
            for i in range(MB5):
                yield from last_rows(2 * i, 2, True)
        _interleave(main(), side, NSUB, MB5)
        for i in range(MB5, NBLK - 1):
            _run(last_rows(2 * i, 2, False))
        _run(last_rows(NT - 2, 1, False))
        _run(last_rows(NT - 1, 1, False))

    def unit(n):
        return n // NT, n % NT

    def load_qm(u):
        qv = qt_ref[u[1], u[0]].astype(BF16)
        zero = jnp.zeros((DH, 128), BF16)
        cols = []
        for h in range(4):
            cols.append(jnp.concatenate(
                [qv[DH * h:DH * (h + 1)] if hh == h else zero for hh in range(4)], axis=0))
        return jnp.concatenate(cols, axis=1)

    def stage_a(u, j, c, qm, mcur, pin):
        nrow = 128 - RC if c < NOFF else 128
        kc = k_ref[u[0], c * HS:c * HS + nrow // 2, :]
        if pin is not None:
            rp = PROW * 8
            mid = jnp.where(pin == pin, kc[rp:rp + 8], jnp.uint32(0))
            kc = jnp.concatenate([kc[:rp], mid, kc[rp + 8:]], axis=0)
        s = jnp.dot(_upk(kc), qm, preferred_element_type=F32)
        s_ref[j, c * 128:c * 128 + nrow, :] = s
        mx = jnp.max(s.reshape(nrow // 8, 8, W), axis=0)
        return mx if mcur is None else jnp.maximum(mcur, mx)

    def vpu_scores(u, j, c, h):
        g, t = u
        kb = kb_ref[g, h * DH:(h + 1) * DH, c * RC:(c + 1) * RC, :].reshape(DH * RC, 128)
        qr = qt_ref[t, g, h * DH:(h + 1) * DH, :]
        sc = None
        for d in range(DH):
            pr = kb[d * RC:(d + 1) * RC] * qr[d:d + 1]
            sc = pr if sc is None else sc + pr
        s_ref[j, (c + 1) * 128 - RC:(c + 1) * 128, h * 128:(h + 1) * 128] = sc
        return jnp.max(sc.reshape(RC // 8, 8, 128), axis=0)

    def stage_b(u, j, c, ms, accs, ls):
        naccs, nls = [], []
        s = s_ref[j, c * 128:(c + 1) * 128, :]
        vt = vt_ref[c, u[0]]
        for h in range(4):
            p = jnp.exp2(s[:, h * 128:(h + 1) * 128].reshape(8, 2, 8, 128) - ms[h])
            pp = jnp.sum(p, axis=1).reshape(64, 128)
            l = None if ls is None else ls[h]
            for r in range(7, -1, -1):
                pr = pp[r * 8:(r + 1) * 8]
                l = pr if l is None else l + pr
            o = jnp.dot(_upk(vt[h * (DH // 2):(h + 1) * (DH // 2)]),
                        p.reshape(128, 128).astype(BF16), preferred_element_type=F32)
            naccs.append(o if accs is None else accs[h] + o)
            nls.append(l)
        return naccs, nls

    def finish(u, accs, ls):
        outs = []
        for h in range(4):
            l = jnp.sum(ls[h], axis=0, keepdims=True)
            outs.append(accs[h] * (1.0 / l))
        ot = jnp.concatenate(outs, axis=0)
        o_ref[u[0], _span(u[1], HS), :] = _pk(ot.T)

    def att_block(b, do_a, do_b):
        pin = None
        for j in range(NSUB):
            n0 = b * NSUB + j
            u = unit(n0)
            ua = unit(n0 + NSUB)
            if do_b:
                if j == 0:
                    up = unit(n0 - 1 if isinstance(n0, int) else jnp.maximum(n0 - 1, 0))
                    finish(up, [a_ref[h * DH:(h + 1) * DH, :] for h in range(4)],
                           [l_ref[h] for h in range(4)])
                mx = jnp.broadcast_to(jnp.max(m_ref[j], axis=0, keepdims=True), (8, W))
                ms = [mx[:, h * 128:(h + 1) * 128].reshape(1, 1, 8, 128) for h in range(4)]
            if do_a:
                qm = load_qm(ua)
            mcur = None
            accs = None
            ls = None
            mv = [None] * 4
            for n, c in enumerate(CHUNK_ORDER):
                if do_b:
                    accs, ls = stage_b(u, j, c, ms, accs, ls)
                if do_a:
                    mcur = stage_a(ua, j, c, qm, mcur, pin)
                    h = (n + 1) % 4
                    mx = vpu_scores(ua, j, n // 4, h)
                    mv[h] = mx if mv[h] is None else jnp.maximum(mv[h], mx)
                    pin = mv[h]
                yield
            if do_a:
                m_ref[j] = jnp.maximum(mcur, jnp.concatenate(mv, axis=1))
            if do_b:
                if j < NSUB - 1 or not do_a:
                    finish(u, accs, ls)
                else:
                    for h in range(4):
                        a_ref[h * DH:(h + 1) * DH, :] = accs[h]
                        l_ref[h] = ls[h]

    def attention():
        a_ref[...] = jnp.zeros(a_ref.shape, F32)
        l_ref[...] = jnp.ones(l_ref.shape, F32)
        gen_keys([(G - 1, 0), (G - 2, 2), (G - 1, 2)])
        _run(att_block(-1, True, False))

        def body(b, c):
            _run(att_block(b, True, True))
            return c
        jax.lax.fori_loop(0, NB - 1, body, 0)
        return att_block(NB - 1, False, True)

    init_a()
    first_phase()
    cp_woa.wait()
    cp_wb.wait()
    cp_wob.wait()

    mid_a()
    init_a()
    phase(mm_ref, proj_b, first=True)
    tail = attention()
    phase(wob_ref, proj_a, side=tail)

    mid_a()
    phase(mm_ref, proj_b)
    tail = attention()
    last_phase(tail)
    out_copy(0, NT).wait()


@jax.jit
def pallas_interleave_layers__linear_attn_block__mha_block__prompt_kernel(
    A_x: jax.Array,
    A_wqkv: jax.Array,
    A_wo: jax.Array,
    B_x: jax.Array,
    B_wqkv: jax.Array,
    B_wo: jax.Array,
):
    del B_x
    x = A_x.reshape(S, D)
    scratch = [
        pltpu.VMEM((S, D), BF16),
        pltpu.VMEM((S, D), F32),
        pltpu.VMEM((D, 3 * D), BF16),
        pltpu.VMEM((D, D), BF16),
        pltpu.VMEM((D, 3 * D), BF16),
        pltpu.VMEM((D, D), BF16),
        pltpu.VMEM((G, S // 2, 128), U32),
        pltpu.VMEM((NT, G, 128, 128), BF16),
        pltpu.VMEM((NT, G, 128, 128), F32),
        pltpu.VMEM((NT, G, 64, 128), U32),
        pltpu.VMEM((G, (S + TM) // 2, 128), U32),
        pltpu.VMEM((G, 128, 128), F32),
        pltpu.VMEM((G, 128, NOFF * RC, 128), F32),
        pltpu.VMEM((G, 128, 128), F32),
        pltpu.VMEM((8, D), F32),
        pltpu.VMEM((D, D), BF16),
        pltpu.VMEM((NSUB, S, W), F32),
        pltpu.VMEM((NSUB, 8, W), F32),
        pltpu.VMEM((128, 128), F32),
        pltpu.VMEM((4, 8, 128), F32),
        pltpu.VMEM((S + TM, D), BF16),
        pltpu.SemaphoreType.DMA((6,)),
        pltpu.SemaphoreType.DMA((NBLK,)),
    ]
    out = pl.pallas_call(
        _kernel,
        out_shape=jax.ShapeDtypeStruct((S, D), BF16),
        in_specs=[pl.BlockSpec(memory_space=pl.ANY)] * 5,
        out_specs=pl.BlockSpec(memory_space=pl.ANY),
        scratch_shapes=scratch,
        compiler_params=pltpu.CompilerParams(vmem_limit_bytes=120 * 1024 * 1024),
    )(x, A_wqkv, A_wo, B_wqkv, B_wo)
    return out.reshape(1, S, D)
```
